```python
import jax
import jax.numpy as jnp

def _softmax(x, axis=-1):
    return jax.nn.softmax(x, axis=axis)

def _gelu(x):
    return jax.nn.gelu(x, approximate=True)

def _silu(x):
    return jax.nn.silu(x)

def _sigmoid(x):
    return jax.nn.sigmoid(x)

def _layernorm(x, axis=-1, eps=1e-05):
    m = jnp.mean(x, axis=axis, keepdims=True)
    v = jnp.var(x, axis=axis, keepdims=True)
    return (x - m) / jnp.sqrt(v + eps)

def _scatter_add(tgt, idx, src, axis=0):
    return tgt.at[idx].add(src)

def _segment_sum(src, seg, n):
    return jax.ops.segment_sum(src, seg, n)

class _Rng:

    def __init__(self, key):
        self._k = key

    def _next(self):
        self._k, sub = jax.random.split(self._k)
        return sub

    def normal(self, shape):
        return jax.random.normal(self._next(), shape, dtype=jnp.bfloat16)

    def randint(self, lo, hi, shape):
        return jax.random.randint(self._next(), shape, lo, hi, dtype=jnp.int32)

    def uniform(self, shape, lo=0.0, hi=1.0):
        return jax.random.uniform(self._next(), shape, jnp.bfloat16, lo, hi)

    def permutation(self, n):
        return jax.random.permutation(self._next(), n)
kernel_name = 'adaLN_cond__sliding_block_cached__moe_arch_mod__prompt'

def setup_inputs():
    _rng = _Rng(jax.random.key(int.from_bytes(__import__("os").urandom(4), "little")))
    _w = lambda a: (lambda t: t.astype(jnp.bfloat16) if jnp.issubdtype(t.dtype, jnp.floating) else t)(jnp.asarray(a))

    def _A_setup():
        B, Sq, D = (1, 2048, 1024)
        Hq, Hkv, Sk, Dh = (32, 4, 2048, 128)
        assert Hq % Hkv == 0, (Hq, Hkv)
        return {'x': _w((lambda *s: _rng.normal(s) * 0.05)(B, Sq, D)), 'k_cache': _w((lambda *s: _rng.normal(s) * 0.05)(B, Hkv, Sk, Dh)), 'v_cache': _w((lambda *s: _rng.normal(s) * 0.05)(B, Hkv, Sk, Dh)), 'wq': _w((lambda *s: _rng.normal(s) * 0.05)(D, Hq * Dh) * D ** (-0.5)), 'wo': _w((lambda *s: _rng.normal(s) * 0.05)(Hq * Dh, D) * (Hq * Dh) ** (-0.5))}
    _A_in = _A_setup()

    def _B_setup():
        B, S, D, F, C = (1, 2048, 1024, 3584, 1)
        return {'x': _w((lambda *s: _rng.normal(s) * 0.05)(B, S, D)), 'w_r': _w((lambda *s: _rng.normal(s) * 0.05)(D)), 'w_gate': _w((lambda *s: _rng.normal(s) * 0.05)(D, F)), 'w_up': _w((lambda *s: _rng.normal(s) * 0.05)(D, F)), 'w_down': _w((lambda *s: _rng.normal(s) * 0.05)(F, D))}
    _B_in = _B_setup()
    return {'A_x': _A_in['x'], 'A_k_cache': _A_in['k_cache'], 'A_v_cache': _A_in['v_cache'], 'A_wq': _A_in['wq'], 'A_wo': _A_in['wo'], 'B_x': _B_in['x'], 'B_w_r': _B_in['w_r'], 'B_w_gate': _B_in['w_gate'], 'B_w_up': _B_in['w_up'], 'B_w_down': _B_in['w_down'], 'c': _w((lambda *s: _rng.normal(s) * 0.05)(1, 1024)), 'w_mod': _w((lambda *s: _rng.normal(s) * 0.05)(1024, 6 * 1024) * 1024 ** (-0.5))}

def reference(A_x, A_k_cache, A_v_cache, A_wq, A_wo, B_x, B_w_r, B_w_gate, B_w_up, B_w_down, c, w_mod):

    def _A_ref(x, k_cache, v_cache, wq, wo):
        B, Sq, D = x.shape
        Hq, Dh = (32, 128)
        Hkv, Sk = (k_cache.shape[1], k_cache.shape[2])
        W = min(4096, max(256, Sk // 4))
        rep = Hq // Hkv
        q = (lambda x, *d: x.transpose(*d))((x @ wq).reshape(B, Sq, Hq, Dh), 0, 2, 1, 3)
        k = jnp.repeat(k_cache[:, :, Sk - W:, :], rep, axis=1)
        v = jnp.repeat(v_cache[:, :, Sk - W:, :], rep, axis=1)
        scores = jnp.einsum('bhqd,bhkd->bhqk', q, k) * Dh ** (-0.5)
        p = _softmax(scores, axis=-1)
        o = jnp.einsum('bhqk,bhkd->bhqd', p, v)
        return (lambda x, *d: x.transpose(*d))(o, 0, 2, 1, 3).reshape(B, Sq, Hq * Dh) @ wo

    def _B_ref(x, w_r, w_gate, w_up, w_down):
        B, S, D = x.shape
        C = 1
        r = x @ w_r
        idx = jnp.argsort(-r, axis=-1)[:, :C]
        idx_e = jnp.repeat(idx.reshape(B, C, 1), D, axis=2)
        x_sel = jnp.take_along_axis(x, idx_e, axis=1)
        g = _silu(x_sel @ w_gate)
        u = x_sel @ w_up
        y = g * u @ w_down
        r_sel = _sigmoid(jnp.take_along_axis(r, idx, axis=1))
        y = y * r_sel.reshape(B, C, 1)
        b_off = (jnp.arange(B) * S).reshape(B, 1)
        flat_idx = (idx + b_off).reshape(B * C)
        zero = (x * 0.0).reshape(B * S, D)
        upd = _scatter_add(zero, flat_idx, y.reshape(B * C, D), axis=0)
        return x + upd.reshape(B, S, D)
    x = A_x
    mod = (_silu(c) @ w_mod).reshape(c.shape[0], 6, 1, -1)
    sa, ca, ga, sb, cb, gb = (mod[:, 0].copy(), mod[:, 1].copy(), mod[:, 2].copy(), mod[:, 3].copy(), mod[:, 4].copy(), mod[:, 5].copy())
    h = _layernorm(x, axis=-1) * (1 + ca) + sa
    x = x + ga * _A_ref(h, A_k_cache, A_v_cache, A_wq, A_wo)
    h = _layernorm(x, axis=-1) * (1 + cb) + sb
    x = x + gb * _B_ref(h, B_w_r, B_w_gate, B_w_up, B_w_down)
    return x
```

```python
import functools

import jax
import jax.numpy as jnp
from jax import lax
from jax.experimental import pallas as pl
from jax.experimental.pallas import tpu as pltpu

_S = 2048
_D = 1024
_HQ = 32
_HKV = 4
_DH = 128
_SK = 2048
_W = min(4096, max(256, _SK // 4))
_F = 3584
_EPS = 1e-5

_M = 256
_NB = _S // _M
_HPS = 4
_NS = _HQ // _HPS
_R = _M // _NS
_QC = _HPS * _DH
_NT = _D // _NS

_LOG2E = 1.4426950408889634
_QSCALE = (_DH ** -0.5) * _LOG2E

_BF = jnp.bfloat16
_F32 = jnp.float32

_SEM_C, _SEM_WR, _SEM_X0, _SEM_XR, _SEM_K, _SEM_V = 0, 1, 2, 3, 4, 5
_SEM_MODA, _SEM_MODB, _SEM_WO, _SEM_WG, _SEM_WU, _SEM_WD = 6, 7, 8, 9, 10, 11
_SEM_OUT, _SEM_FIX = 12, 13
_SEM_WQ = 14
_NSEM = _SEM_WQ + _NS


def _kernel(x_hbm, k_hbm, v_hbm, wq_hbm, wo_hbm, wr_hbm, wg_hbm, wu_hbm, wd_hbm, c_hbm, wmod_hbm,
            out_hbm,
            x_v, h_v, k_v, kT_v, v_v, wq_v, wo_v, wmod_v, wg_v, wu_v, wd_v, c_v, wr_v,
            q_v, o_v, a_v, out_v, h2_v, of_v, mod_v, best_v, bidx_v, fix_v, sems):

    def cp(src, dst, slot):
        return pltpu.make_async_copy(src, dst, sems.at[slot])

    d_c = cp(c_hbm, c_v, _SEM_C)
    d_x0 = cp(x_hbm.at[pl.ds(0, 2 * _M)], x_v.at[pl.ds(0, 2 * _M)], _SEM_X0)
    d_moda = cp(wmod_hbm.at[:, pl.ds(0, 2 * _D)], wmod_v.at[:, pl.ds(0, 2 * _D)], _SEM_MODA)
    d_k = cp(k_hbm.at[:, pl.ds(_SK - _W, _W), :], k_v, _SEM_K)
    d_v = cp(v_hbm.at[:, pl.ds(_SK - _W, _W), :], v_v, _SEM_V)

    def d_wq(j):
        return cp(wq_hbm.at[:, pl.ds(pl.multiple_of(j * _QC, _QC), _QC)], wq_v.at[j], _SEM_WQ + j)

    d_xr = cp(x_hbm.at[pl.ds(2 * _M, _S - 2 * _M)], x_v.at[pl.ds(2 * _M, _S - 2 * _M)], _SEM_XR)
    d_wr = cp(wr_hbm, wr_v, _SEM_WR)
    d_modb = cp(wmod_hbm.at[:, pl.ds(2 * _D, 4 * _D)], wmod_v.at[:, pl.ds(2 * _D, 4 * _D)], _SEM_MODB)
    d_wg = cp(wg_hbm, wg_v, _SEM_WG)
    d_wu = cp(wu_hbm, wu_v, _SEM_WU)
    d_wd = cp(wd_hbm, wd_v, _SEM_WD)

    d_c.start()
    d_x0.start()
    d_moda.start()
    d_wq(0).start()
    d_k.start()
    d_v.start()
    d_wq(1).start()
    d_xr.start()
    for j in range(2, _NS):
        d_wq(j).start()
    for j in range(_NS):
        cp(wo_hbm.at[:, pl.ds(j * _NT, _NT)], wo_v.at[j], _SEM_WO).start()
    d_wr.start()
    d_modb.start()
    d_wg.start()
    d_wu.start()
    d_wd.start()

    def mod_chunk(i):
        cb16 = c_v[...].astype(_F32)
        sc = (cb16 * jax.nn.sigmoid(cb16)).astype(_BF)
        sc = jnp.broadcast_to(sc, (16, _D))
        m = jnp.dot(sc, wmod_v[:, pl.ds(i * _D, _D)], preferred_element_type=_F32)
        return m[0:8, :]

    def modr(i):
        return mod_v[i, 0:1, :]

    def ln(xf):
        mu = jnp.mean(xf, axis=1, keepdims=True)
        d = xf - mu
        var = jnp.mean(d * d, axis=1, keepdims=True)
        return d * lax.rsqrt(var + _EPS)

    def ln1_slice(u):
        rows = pl.ds(pl.multiple_of(u * _R, _R), _R)
        y = ln(x_v[rows, :].astype(_F32))
        h = y * modr(1) + modr(0)
        h_v[rows, :] = h.astype(_BF)

    def qproj(t, slot):
        b = t // _NS
        j = t % _NS
        rows = pl.ds(pl.multiple_of(b * _M, _M), _M)
        q = jnp.dot(h_v[rows, :], wq_v[j], preferred_element_type=_F32)
        q_v[slot] = q.astype(_BF)

    def attention(t):
        b = t // _NS
        j = t % _NS
        g = j // 2
        for hh in range(_HPS):
            q = q_v[t % 2, :, pl.ds(hh * _DH, _DH)]
            s = jnp.dot(q, kT_v[g], preferred_element_type=_F32)
            m = jnp.max(s, axis=1, keepdims=True)
            p = jnp.exp2(s - m)
            l = jnp.sum(p, axis=1, keepdims=True)
            o = jnp.dot(p.astype(_BF), v_v[g], preferred_element_type=_F32)
            o_v[b % 2, j, :, pl.ds(hh * _DH, _DH)] = (o * (1.0 / l)).astype(_BF)

    def oproj(b, j):
        lhs = jnp.concatenate([o_v[b % 2, jj] for jj in range(_NS)], axis=1)
        a_v[b % 2, j] = jnp.dot(lhs, wo_v[j], preferred_element_type=_F32)

    def epilogue(b, i):
        lrows = pl.ds(pl.multiple_of(i * _R, _R), _R)
        row0 = pl.multiple_of(b * _M + i * _R, _R)
        rows = pl.ds(row0, _R)
        a = jnp.concatenate([a_v[b % 2, jj, lrows, :] for jj in range(_NS)], axis=1)
        x1 = x_v[rows, :].astype(_F32) + modr(2) * a
        h2 = ln(x1) * modr(4) + modr(3)
        o = x1 + modr(5) * h2
        out_v[rows, :] = o.astype(_BF)
        h2_v[rows, :] = h2
        of_v[rows, :] = o
        r = jnp.sum(h2 * wr_v[...].astype(_F32), axis=1, keepdims=True)
        r = jnp.broadcast_to(r, (_R, 128))
        ridx = row0 + lax.broadcasted_iota(jnp.int32, (_R, 128), 0)
        bv = best_v[...]
        bi = bidx_v[...]
        for s in range(_R // 8):
            rs = r[s * 8:(s + 1) * 8]
            upd = rs > bv
            bv = jnp.where(upd, rs, bv)
            bi = jnp.where(upd, ridx[s * 8:(s + 1) * 8], bi)
        best_v[...] = bv
        bidx_v[...] = bi

    def block_phase(b, do_attn, do_q_last, do_o, do_epi, wait_wq):
        def step(j, carry):
            t = b * _NS + j
            if do_epi:
                epilogue(b - 2, j)
            if do_o:
                oproj(b - 1, j)
            if do_attn:
                attention(t)
                if wait_wq:
                    @pl.when(j + 1 < _NS)
                    def _():
                        d_wq(j + 1).wait()
                qproj(t + 1 if do_q_last else jnp.minimum(t + 1, _NB * _NS - 1), (t + 1) % 2)
                ln1_slice(jnp.minimum(t + _NS + 1, _NB * _NS - 1))
            return carry
        lax.fori_loop(0, _NS, step, 0)

    def out_copy(b):
        rows = pl.ds(pl.multiple_of(b * _M, _M), _M)
        return cp(out_v.at[rows], out_hbm.at[rows], _SEM_OUT)

    d_c.wait()
    d_moda.wait()
    mod_v[0] = mod_chunk(0) * _QSCALE
    mod_v[1] = (1.0 + mod_chunk(1)) * _QSCALE
    d_x0.wait()
    for u in range(_NS + 1):
        ln1_slice(u)
    d_wq(0).wait()
    qproj(0, 0)
    d_k.wait()
    for g in range(_HKV):
        kT_v[g] = k_v[g].astype(_F32).T.astype(_BF)
    d_v.wait()
    d_xr.wait()
    best_v[...] = jnp.full((8, 128), -jnp.inf, _F32)
    bidx_v[...] = jnp.zeros((8, 128), jnp.int32)

    block_phase(0, True, True, False, False, True)

    pltpu.make_async_copy(wo_v, wo_v, sems.at[_SEM_WO]).wait()
    d_wr.wait()
    d_modb.wait()
    mod_v[2] = mod_chunk(2)
    mod_v[3] = mod_chunk(3)
    mod_v[4] = 1.0 + mod_chunk(4)
    mod_v[5] = mod_chunk(5)

    block_phase(1, True, True, True, False, False)

    def main_block(b, carry):
        block_phase(b, True, True, True, True, False)
        out_copy(b - 2).start()
        return carry
    lax.fori_loop(2, _NB - 1, main_block, 0)

    block_phase(_NB - 1, True, False, True, True, False)
    out_copy(_NB - 3).start()
    block_phase(_NB, False, False, True, True, False)
    out_copy(_NB - 2).start()
    block_phase(_NB + 1, False, False, False, True, False)
    out_copy(_NB - 1).start()

    bv = best_v[...]
    bi = bidx_v[...]
    rmax = jnp.max(bv, axis=0, keepdims=True)
    cand = jnp.where(bv == rmax, bi, _S)
    sel = jnp.min(cand)
    sel = jnp.clip(sel, 0, _S - 1)
    gate_r = jax.nn.sigmoid(rmax[:, 0:1])

    xs = h2_v[pl.ds(sel, 1), :].astype(_BF)
    xs = jnp.broadcast_to(xs, (16, _D))
    d_wg.wait()
    d_wu.wait()
    g = jnp.dot(xs, wg_v[...], preferred_element_type=_F32)
    u = jnp.dot(xs, wu_v[...], preferred_element_type=_F32)
    act = (g * jax.nn.sigmoid(g) * u).astype(_BF)
    d_wd.wait()
    y = jnp.dot(act, wd_v[...], preferred_element_type=_F32)[0:1, :]
    row = of_v[pl.ds(sel, 1), :] + modr(5) * (y * gate_r)

    base = pl.multiple_of((sel // 16) * 16, 16)
    tile = of_v[pl.ds(base, 16), :]
    rid = base + lax.broadcasted_iota(jnp.int32, (16, _D), 0)
    fix_v[...] = jnp.where(rid == sel, row, tile).astype(_BF)

    pltpu.make_async_copy(out_v, out_hbm, sems.at[_SEM_OUT]).wait()
    d_fix = cp(fix_v, out_hbm.at[pl.ds(base, 16)], _SEM_FIX)
    d_fix.start()
    d_fix.wait()


@jax.jit
def pallas_adaLN_cond__sliding_block_cached__moe_arch_mod__prompt_kernel(
    A_x: jax.Array,
    A_k_cache: jax.Array,
    A_v_cache: jax.Array,
    A_wq: jax.Array,
    A_wo: jax.Array,
    B_x: jax.Array,
    B_w_r: jax.Array,
    B_w_gate: jax.Array,
    B_w_up: jax.Array,
    B_w_down: jax.Array,
    c: jax.Array,
    w_mod: jax.Array,
):
    del B_x
    x = A_x.reshape(_S, _D)
    k = A_k_cache.reshape(_HKV, _SK, _DH)
    v = A_v_cache.reshape(_HKV, _SK, _DH)
    wr = B_w_r.reshape(1, _D)

    any_spec = pl.BlockSpec(memory_space=pl.ANY)
    out = pl.pallas_call(
        _kernel,
        out_shape=jax.ShapeDtypeStruct((_S, _D), _BF),
        in_specs=[any_spec] * 11,
        out_specs=any_spec,
        scratch_shapes=[
            pltpu.VMEM((_S, _D), _BF),
            pltpu.VMEM((_S, _D), _BF),
            pltpu.VMEM((_HKV, _W, _DH), _BF),
            pltpu.VMEM((_HKV, _DH, _W), _BF),
            pltpu.VMEM((_HKV, _W, _DH), _BF),
            pltpu.VMEM((_NS, _D, _QC), _BF),
            pltpu.VMEM((_NS, _HQ * _DH, _NT), _BF),
            pltpu.VMEM((_D, 6 * _D), _BF),
            pltpu.VMEM((_D, _F), _BF),
            pltpu.VMEM((_D, _F), _BF),
            pltpu.VMEM((_F, _D), _BF),
            pltpu.VMEM((1, _D), _BF),
            pltpu.VMEM((1, _D), _BF),
            pltpu.VMEM((2, _M, _QC), _BF),
            pltpu.VMEM((2, _NS, _M, _QC), _BF),
            pltpu.VMEM((2, _NS, _M, _NT), _F32),
            pltpu.VMEM((_S, _D), _BF),
            pltpu.VMEM((_S, _D), _F32),
            pltpu.VMEM((_S, _D), _F32),
            pltpu.VMEM((6, 8, _D), _F32),
            pltpu.VMEM((8, 128), _F32),
            pltpu.VMEM((8, 128), jnp.int32),
            pltpu.VMEM((16, _D), _BF),
            pltpu.SemaphoreType.DMA((_NSEM,)),
        ],
        compiler_params=pltpu.CompilerParams(vmem_limit_bytes=110 * 1024 * 1024),
    )(x, k, v, A_wq, A_wo, wr, B_w_gate, B_w_up, B_w_down, c, w_mod)
    return out.reshape(1, _S, _D)
```

```python
import functools

import jax
import jax.numpy as jnp
from jax import lax
from jax.experimental import pallas as pl
from jax.experimental.pallas import tpu as pltpu

_S = 2048
_D = 1024
_HQ = 32
_HKV = 4
_DH = 128
_SK = 2048
_W = min(4096, max(256, _SK // 4))
_F = 3584
_EPS = 1e-5

_M = 512
_NB = _S // _M
_HPS = 4
_NS = _HQ // _HPS
_R = _M // _NS
_QC = _HPS * _DH
_NT = _D // _NS
_SPG = _NS // _HKV

_LOG2E = 1.4426950408889634
_QSCALE = (_DH ** -0.5) * _LOG2E

_BF = jnp.bfloat16
_F32 = jnp.float32

_SEM_C, _SEM_WR, _SEM_K, _SEM_V = 0, 1, 2, 3
_SEM_MODA, _SEM_MODB, _SEM_WO, _SEM_WG, _SEM_WU, _SEM_WD = 4, 5, 6, 7, 8, 9
_SEM_OUT, _SEM_FIX = 10, 11
_SEM_WQ = 12
_SEM_X = _SEM_WQ + _NS
_NSEM = _SEM_X + _NB


def _kernel(x_hbm, k_hbm, v_hbm, wq_hbm, wo_hbm, wr_hbm, wg_hbm, wu_hbm, wd_hbm, c_hbm, wmod_hbm,
            out_hbm,
            x_v, h_a, h_b, k_v, kT_v, v_v, wq_v, wo_v, wmod_v, wg_v, wu_v, wd_v, c_v, wr_v,
            o_a, o_b, a_a, a_b, out_v, h2_v, of_v, mod_v, best_v, bidx_v, fix_v, sems):
    h_buf, o_buf, a_buf = (h_a, h_b), (o_a, o_b), (a_a, a_b)

    def cp(src, dst, slot):
        return pltpu.make_async_copy(src, dst, sems.at[slot])

    d_c = cp(c_hbm, c_v, _SEM_C)
    d_moda = cp(wmod_hbm.at[:, pl.ds(0, 2 * _D)], wmod_v.at[:, pl.ds(0, 2 * _D)], _SEM_MODA)
    d_k = cp(k_hbm.at[:, pl.ds(_SK - _W, _W), :], k_v, _SEM_K)
    d_v = cp(v_hbm.at[:, pl.ds(_SK - _W, _W), :], v_v, _SEM_V)

    def d_wq(j):
        return cp(wq_hbm.at[:, pl.ds(pl.multiple_of(j * _QC, _QC), _QC)], wq_v.at[j], _SEM_WQ + j)

    def d_x(b):
        return cp(x_hbm.at[pl.ds(b * _M, _M)], x_v.at[pl.ds(b * _M, _M)], _SEM_X + b)

    d_wr = cp(wr_hbm, wr_v, _SEM_WR)
    d_modb = cp(wmod_hbm.at[:, pl.ds(2 * _D, 4 * _D)], wmod_v.at[:, pl.ds(2 * _D, 4 * _D)], _SEM_MODB)
    d_wg = cp(wg_hbm, wg_v, _SEM_WG)
    d_wu = cp(wu_hbm, wu_v, _SEM_WU)
    d_wd = cp(wd_hbm, wd_v, _SEM_WD)

    d_c.start()
    d_x(0).start()
    d_moda.start()
    d_wq(0).start()
    d_k.start()
    d_v.start()
    d_x(1).start()
    for j in range(1, _NS):
        d_wq(j).start()
    for j in range(_NS):
        cp(wo_hbm.at[:, pl.ds(j * _NT, _NT)], wo_v.at[j], _SEM_WO).start()
    for b in range(2, _NB):
        d_x(b).start()
    d_wr.start()
    d_modb.start()
    d_wg.start()
    d_wu.start()
    d_wd.start()

    def mod_chunk(i):
        cb16 = c_v[...].astype(_F32)
        sc = (cb16 * jax.nn.sigmoid(cb16)).astype(_BF)
        sc = jnp.broadcast_to(sc, (16, _D))
        m = jnp.dot(sc, wmod_v[:, pl.ds(i * _D, _D)], preferred_element_type=_F32)
        return m[0:8, :]

    def modr(i):
        return mod_v[i, 0:1, :]

    def ln(xf):
        mu = jnp.mean(xf, axis=1, keepdims=True)
        d = xf - mu
        var = jnp.mean(d * d, axis=1, keepdims=True)
        return d * lax.rsqrt(var + _EPS)

    def ln1_slice(b, i):
        lrows = pl.ds(pl.multiple_of(i * _R, _R), _R)
        rows = pl.ds(pl.multiple_of(b * _M + i * _R, _R), _R)
        y = ln(x_v[rows, :].astype(_F32))
        h = y * modr(1) + modr(0)
        h_buf[b % 2][lrows, :] = h.astype(_BF)

    def qproj_head(b, j, hh):
        q = jnp.dot(h_buf[b % 2][...], wq_v[j, :, pl.ds(hh * _DH, _DH)],
                    preferred_element_type=_F32)
        return q.astype(_BF)

    def scores(j, q):
        return jnp.dot(q, kT_v[j // _SPG], preferred_element_type=_F32)

    def softmax_pv(b, j, hh, s):
        m = jnp.max(s, axis=1, keepdims=True)
        p = jnp.exp2(s - m)
        l = jnp.sum(p, axis=1, keepdims=True)
        o = jnp.dot(p.astype(_BF), v_v[j // _SPG], preferred_element_type=_F32)
        o_buf[b % 2][j, :, pl.ds(hh * _DH, _DH)] = (o * (1.0 / l)).astype(_BF)

    def oproj_part(b, j, part):
        n = _NS // _HPS
        lhs = jnp.concatenate([o_buf[b % 2][part * n + jj] for jj in range(n)], axis=1)
        return jnp.dot(lhs, wo_v[j, pl.ds(part * n * _QC, n * _QC), :], preferred_element_type=_F32)

    def epilogue(b, i):
        lrows = pl.ds(pl.multiple_of(i * _R, _R), _R)
        row0 = pl.multiple_of(b * _M + i * _R, _R)
        rows = pl.ds(row0, _R)
        a = jnp.concatenate([a_buf[b % 2][jj, lrows, :] for jj in range(_NS)], axis=1)
        x1 = x_v[rows, :].astype(_F32) + modr(2) * a
        h2 = ln(x1) * modr(4) + modr(3)
        o = x1 + modr(5) * h2
        out_v[rows, :] = o.astype(_BF)
        h2_v[rows, :] = h2
        of_v[rows, :] = o
        r = jnp.sum(h2 * wr_v[...].astype(_F32), axis=1, keepdims=True)
        r = jnp.broadcast_to(r, (_R, 128))
        ridx = row0 + lax.broadcasted_iota(jnp.int32, (_R, 128), 0)
        bv = best_v[...]
        bi = bidx_v[...]
        for s in range(_R // 8):
            rs = r[s * 8:(s + 1) * 8]
            upd = rs > bv
            bv = jnp.where(upd, rs, bv)
            bi = jnp.where(upd, ridx[s * 8:(s + 1) * 8], bi)
        best_v[...] = bv
        bidx_v[...] = bi

    def block_phase(b):
        do_attn = b < _NB
        do_o = 0 <= b - 1 < _NB
        do_epi = 0 <= b - 2
        do_ln = b + 1 < _NB

        def step(j, carry):
            if do_epi:
                epilogue(b - 2, j)
            if b == 0:
                d_wq(j).wait()
            parts = []
            if do_attn:
                q = qproj_head(b, j, 0)
            for hh in range(_HPS):
                if do_o and hh in (0, _HPS - 1):
                    if hh == 0:
                        parts.append(oproj_part(b - 1, j, 0))
                if do_attn:
                    s = scores(j, q)
                    if hh + 1 < _HPS:
                        q = qproj_head(b, j, hh + 1)
                    elif do_o:
                        parts.append(oproj_part(b - 1, j, 1))
                    softmax_pv(b, j, hh, s)
            if do_o:
                for part in range(len(parts), _HPS):
                    parts.append(oproj_part(b - 1, j, part))
                a_buf[(b - 1) % 2][j] = functools.reduce(lambda u, w: u + w, parts)
            if do_ln:
                ln1_slice(b + 1, j)
            return carry
        lax.fori_loop(0, _NS, step, 0)

    def out_copy(b):
        rows = pl.ds(b * _M, _M)
        return cp(out_v.at[rows], out_hbm.at[rows], _SEM_OUT)

    d_c.wait()
    d_moda.wait()
    mod_v[0] = mod_chunk(0) * _QSCALE
    mod_v[1] = (1.0 + mod_chunk(1)) * _QSCALE
    d_x(0).wait()
    for i in range(_NS):
        ln1_slice(0, i)
    d_k.wait()
    for g in range(_HKV):
        kT_v[g] = k_v[g].astype(_F32).T.astype(_BF)
    d_v.wait()
    best_v[...] = jnp.full((8, 128), -jnp.inf, _F32)
    bidx_v[...] = jnp.zeros((8, 128), jnp.int32)

    for b in range(_NB + 2):
        if b == 1:
            pltpu.make_async_copy(wo_v, wo_v, sems.at[_SEM_WO]).wait()
            d_wr.wait()
            d_modb.wait()
            mod_v[2] = mod_chunk(2)
            mod_v[3] = mod_chunk(3)
            mod_v[4] = 1.0 + mod_chunk(4)
            mod_v[5] = mod_chunk(5)
        if b + 1 < _NB:
            d_x(b + 1).wait()
        block_phase(b)
        if b >= 2:
            out_copy(b - 2).start()

    bv = best_v[...]
    bi = bidx_v[...]
    rmax = jnp.max(bv, axis=0, keepdims=True)
    cand = jnp.where(bv == rmax, bi, _S)
    sel = jnp.min(cand)
    sel = jnp.clip(sel, 0, _S - 1)
    gate_r = jax.nn.sigmoid(rmax[:, 0:1])

    xs = h2_v[pl.ds(sel, 1), :].astype(_BF)
    xs = jnp.broadcast_to(xs, (16, _D))
    d_wg.wait()
    d_wu.wait()
    g = jnp.dot(xs, wg_v[...], preferred_element_type=_F32)
    u = jnp.dot(xs, wu_v[...], preferred_element_type=_F32)
    act = (g * jax.nn.sigmoid(g) * u).astype(_BF)
    d_wd.wait()
    y = jnp.dot(act, wd_v[...], preferred_element_type=_F32)[0:1, :]
    row = of_v[pl.ds(sel, 1), :] + modr(5) * (y * gate_r)

    base = pl.multiple_of((sel // 16) * 16, 16)
    tile = of_v[pl.ds(base, 16), :]
    rid = base + lax.broadcasted_iota(jnp.int32, (16, _D), 0)
    fix_v[...] = jnp.where(rid == sel, row, tile).astype(_BF)

    pltpu.make_async_copy(out_v, out_hbm, sems.at[_SEM_OUT]).wait()
    d_fix = cp(fix_v, out_hbm.at[pl.ds(base, 16)], _SEM_FIX)
    d_fix.start()
    d_fix.wait()


@jax.jit
def pallas_adaLN_cond__sliding_block_cached__moe_arch_mod__prompt_kernel(
    A_x: jax.Array,
    A_k_cache: jax.Array,
    A_v_cache: jax.Array,
    A_wq: jax.Array,
    A_wo: jax.Array,
    B_x: jax.Array,
    B_w_r: jax.Array,
    B_w_gate: jax.Array,
    B_w_up: jax.Array,
    B_w_down: jax.Array,
    c: jax.Array,
    w_mod: jax.Array,
):
    del B_x
    x = A_x.reshape(_S, _D)
    k = A_k_cache.reshape(_HKV, _SK, _DH)
    v = A_v_cache.reshape(_HKV, _SK, _DH)
    wr = B_w_r.reshape(1, _D)

    any_spec = pl.BlockSpec(memory_space=pl.ANY)
    out = pl.pallas_call(
        _kernel,
        out_shape=jax.ShapeDtypeStruct((_S, _D), _BF),
        in_specs=[any_spec] * 11,
        out_specs=any_spec,
        scratch_shapes=[
            pltpu.VMEM((_S, _D), _BF),
            pltpu.VMEM((_M, _D), _BF),
            pltpu.VMEM((_M, _D), _BF),
            pltpu.VMEM((_HKV, _W, _DH), _BF),
            pltpu.VMEM((_HKV, _DH, _W), _BF),
            pltpu.VMEM((_HKV, _W, _DH), _BF),
            pltpu.VMEM((_NS, _D, _QC), _BF),
            pltpu.VMEM((_NS, _HQ * _DH, _NT), _BF),
            pltpu.VMEM((_D, 6 * _D), _BF),
            pltpu.VMEM((_D, _F), _BF),
            pltpu.VMEM((_D, _F), _BF),
            pltpu.VMEM((_F, _D), _BF),
            pltpu.VMEM((1, _D), _BF),
            pltpu.VMEM((1, _D), _BF),
            pltpu.VMEM((_NS, _M, _QC), _BF),
            pltpu.VMEM((_NS, _M, _QC), _BF),
            pltpu.VMEM((_NS, _M, _NT), _F32),
            pltpu.VMEM((_NS, _M, _NT), _F32),
            pltpu.VMEM((_S, _D), _BF),
            pltpu.VMEM((_S, _D), _F32),
            pltpu.VMEM((_S, _D), _F32),
            pltpu.VMEM((6, 8, _D), _F32),
            pltpu.VMEM((8, 128), _F32),
            pltpu.VMEM((8, 128), jnp.int32),
            pltpu.VMEM((16, _D), _BF),
            pltpu.SemaphoreType.DMA((_NSEM,)),
        ],
        compiler_params=pltpu.CompilerParams(vmem_limit_bytes=110 * 1024 * 1024),
    )(x, k, v, A_wq, A_wo, wr, B_w_gate, B_w_up, B_w_down, c, w_mod)
    return out.reshape(1, _S, _D)
```

```python
import functools

import jax
import jax.numpy as jnp
from jax import lax
from jax.experimental import pallas as pl
from jax.experimental.pallas import tpu as pltpu

_S = 2048
_D = 1024
_HQ = 32
_HKV = 4
_DH = 128
_SK = 2048
_W = min(4096, max(256, _SK // 4))
_F = 3584
_EPS = 1e-5

_M = 512
_NB = _S // _M
_HPS = 4
_NS = _HQ // _HPS
_R = _M // _NS
_QC = _HPS * _DH
_NT = _D // _NS
_SPG = _NS // _HKV

_LOG2E = 1.4426950408889634
_QSCALE = (_DH ** -0.5) * _LOG2E

_BF = jnp.bfloat16
_F32 = jnp.float32

_SEM_C, _SEM_WR, _SEM_K, _SEM_V = 0, 1, 2, 3
_SEM_MODA, _SEM_MODB, _SEM_WO, _SEM_WG, _SEM_WU, _SEM_WD = 4, 5, 6, 7, 8, 9
_SEM_OUT, _SEM_FIX = 10, 11
_SEM_WQ = 12
_SEM_X = _SEM_WQ + _NS
_NSEM = _SEM_X + _NB


def _kernel(x_hbm, k_hbm, v_hbm, wq_hbm, wo_hbm, wr_hbm, wg_hbm, wu_hbm, wd_hbm, c_hbm, wmod_hbm,
            out_hbm,
            x_v, h_a, h_b, k_v, kT_v, v_v, vv_v, wq_v, wo_v, wmod_v, wg_v, wu_v, wd_v, c_v, wr_v,
            o_a, o_b, a_a, a_b, out_v, h2_v, of_v, mod_v, best_v, bidx_v, fix_v, sems):
    h_buf, o_buf, a_buf = (h_a, h_b), (o_a, o_b), (a_a, a_b)

    def cp(src, dst, slot):
        return pltpu.make_async_copy(src, dst, sems.at[slot])

    d_c = cp(c_hbm, c_v, _SEM_C)
    d_moda = cp(wmod_hbm.at[:, pl.ds(0, 2 * _D)], wmod_v.at[:, pl.ds(0, 2 * _D)], _SEM_MODA)
    d_k = cp(k_hbm.at[:, pl.ds(_SK - _W, _W), :], k_v, _SEM_K)
    d_v = cp(v_hbm.at[:, pl.ds(_SK - _W, _W), :], v_v, _SEM_V)

    def d_wq(j):
        return cp(wq_hbm.at[:, pl.ds(pl.multiple_of(j * _QC, _QC), _QC)], wq_v.at[j], _SEM_WQ + j)

    def d_x(b):
        return cp(x_hbm.at[pl.ds(b * _M, _M)], x_v.at[pl.ds(b * _M, _M)], _SEM_X + b)

    d_wr = cp(wr_hbm, wr_v, _SEM_WR)
    d_modb = cp(wmod_hbm.at[:, pl.ds(2 * _D, 4 * _D)], wmod_v.at[:, pl.ds(2 * _D, 4 * _D)], _SEM_MODB)
    d_wg = cp(wg_hbm, wg_v, _SEM_WG)
    d_wu = cp(wu_hbm, wu_v, _SEM_WU)
    d_wd = cp(wd_hbm, wd_v, _SEM_WD)

    d_c.start()
    d_x(0).start()
    d_moda.start()
    d_wq(0).start()
    d_k.start()
    d_v.start()
    d_x(1).start()
    for j in range(1, _NS):
        d_wq(j).start()
    for j in range(_NS):
        cp(wo_hbm.at[:, pl.ds(j * _NT, _NT)], wo_v.at[j], _SEM_WO).start()
    for b in range(2, _NB):
        d_x(b).start()
    d_wr.start()
    d_modb.start()
    d_wg.start()
    d_wu.start()
    d_wd.start()

    def mod_chunk(i):
        cb16 = c_v[...].astype(_F32)
        sc = (cb16 * jax.nn.sigmoid(cb16)).astype(_BF)
        sc = jnp.broadcast_to(sc, (16, _D))
        m = jnp.dot(sc, wmod_v[:, pl.ds(i * _D, _D)], preferred_element_type=_F32)
        return m[0:8, :]

    def modr(i):
        return mod_v[i, 0:1, :]

    def pack(xf):
        return pltpu.bitcast(xf.astype(_BF), jnp.uint32)

    def unpack(w):
        return pltpu.bitcast(w, _BF)

    def ln(xf):
        mu = jnp.mean(xf, axis=1, keepdims=True)
        d = xf - mu
        var = jnp.mean(d * d, axis=1, keepdims=True)
        return d * lax.rsqrt(var + _EPS)

    def ln1_slice(b, i):
        rows = pl.ds(pl.multiple_of(b * _M + i * _R, _R), _R)
        y = ln(x_v[rows, :].astype(_F32))
        h = y * modr(1) + modr(0)
        h_buf[b % 2][pl.ds(pl.multiple_of(i * (_R // 2), _R // 2), _R // 2), :] = pack(h)

    def qproj_head(b, j, hh):
        q = jnp.dot(unpack(h_buf[b % 2][...]), wq_v[j, :, pl.ds(hh * _DH, _DH)],
                    preferred_element_type=_F32)
        return q.astype(_BF)

    def scores(j, q):
        return jnp.dot(q, unpack(kT_v[j // _SPG]), preferred_element_type=_F32)

    def softmax_pv(b, j, hh, s):
        m = jnp.max(s, axis=1, keepdims=True)
        p = jnp.exp2(s - m)
        l = jnp.sum(p, axis=1, keepdims=True)
        o = jnp.dot(p.astype(_BF), unpack(vv_v[j // _SPG]), preferred_element_type=_F32)
        r = pl.reciprocal(l, approx=True)
        r = r * (2.0 - l * r)
        o_buf[b % 2][j, :, pl.ds(hh * _DH, _DH)] = pack(o * r)

    def oproj_part(b, j, part):
        n = _NS // _HPS
        lhs = jnp.concatenate([unpack(o_buf[b % 2][part * n + jj]) for jj in range(n)], axis=1)
        return jnp.dot(lhs, wo_v[j, pl.ds(part * n * _QC, n * _QC), :], preferred_element_type=_F32)

    def epilogue(b, i):
        lrows = pl.ds(pl.multiple_of(i * _R, _R), _R)
        row0 = pl.multiple_of(b * _M + i * _R, _R)
        rows = pl.ds(row0, _R)
        a = jnp.concatenate([a_buf[b % 2][jj, lrows, :] for jj in range(_NS)], axis=1)
        x1 = x_v[rows, :].astype(_F32) + modr(2) * a
        h2 = ln(x1) * modr(4) + modr(3)
        o = x1 + modr(5) * h2
        out_v[rows, :] = o.astype(_BF)
        h2_v[rows, :] = h2
        of_v[rows, :] = o
        r = jnp.sum(h2 * wr_v[...].astype(_F32), axis=1, keepdims=True)
        r = jnp.broadcast_to(r, (_R, 128))
        ridx = row0 + lax.broadcasted_iota(jnp.int32, (_R, 128), 0)
        bv = best_v[...]
        bi = bidx_v[...]
        for s in range(_R // 8):
            rs = r[s * 8:(s + 1) * 8]
            upd = rs > bv
            bv = jnp.where(upd, rs, bv)
            bi = jnp.where(upd, ridx[s * 8:(s + 1) * 8], bi)
        best_v[...] = bv
        bidx_v[...] = bi

    def block_phase(b):
        do_attn = b < _NB
        do_o = 0 <= b - 1 < _NB
        do_epi = 0 <= b - 2
        do_ln = b + 1 < _NB

        def step(j, carry):
            if b == 0:
                d_wq(j).wait()
            parts = []
            if do_attn:
                q = qproj_head(b, j, 0)
            for hh in range(_HPS):
                if do_o and hh in (0, _HPS - 1):
                    if hh == 0:
                        parts.append(oproj_part(b - 1, j, 0))
                if do_attn:
                    s = scores(j, q)
                    if hh + 1 < _HPS:
                        q = qproj_head(b, j, hh + 1)
                    elif do_o:
                        parts.append(oproj_part(b - 1, j, 1))
                    softmax_pv(b, j, hh, s)
            if do_epi:
                epilogue(b - 2, j)
            if do_ln:
                ln1_slice(b + 1, j)
            if do_o:
                for part in range(len(parts), _HPS):
                    parts.append(oproj_part(b - 1, j, part))
                a_buf[(b - 1) % 2][j] = functools.reduce(lambda u, w: u + w, parts)
            return carry
        lax.fori_loop(0, _NS, step, 0)

    def out_copy(b):
        rows = pl.ds(b * _M, _M)
        return cp(out_v.at[rows], out_hbm.at[rows], _SEM_OUT)

    d_c.wait()
    d_moda.wait()
    mod_v[0] = mod_chunk(0) * _QSCALE
    mod_v[1] = (1.0 + mod_chunk(1)) * _QSCALE
    d_x(0).wait()
    for i in range(_NS):
        ln1_slice(0, i)
    d_k.wait()
    for g in range(_HKV):
        kT_v[g] = pack(k_v[g].astype(_F32).T)
    d_v.wait()
    for g in range(_HKV):
        vv_v[g] = pltpu.bitcast(v_v[g], jnp.uint32)
    best_v[...] = jnp.full((8, 128), -jnp.inf, _F32)
    bidx_v[...] = jnp.zeros((8, 128), jnp.int32)

    for b in range(_NB + 2):
        if b == 1:
            pltpu.make_async_copy(wo_v, wo_v, sems.at[_SEM_WO]).wait()
            d_wr.wait()
            d_modb.wait()
            mod_v[2] = mod_chunk(2)
            mod_v[3] = mod_chunk(3)
            mod_v[4] = 1.0 + mod_chunk(4)
            mod_v[5] = mod_chunk(5)
        if b + 1 < _NB:
            d_x(b + 1).wait()
        block_phase(b)
        if b >= 2:
            out_copy(b - 2).start()

    bv = best_v[...]
    bi = bidx_v[...]
    rmax = jnp.max(bv, axis=0, keepdims=True)
    cand = jnp.where(bv == rmax, bi, _S)
    sel = jnp.min(cand)
    sel = jnp.clip(sel, 0, _S - 1)
    gate_r = jax.nn.sigmoid(rmax[:, 0:1])

    xs = h2_v[pl.ds(sel, 1), :].astype(_BF)
    xs = jnp.broadcast_to(xs, (16, _D))
    d_wg.wait()
    d_wu.wait()
    g = jnp.dot(xs, wg_v[...], preferred_element_type=_F32)
    u = jnp.dot(xs, wu_v[...], preferred_element_type=_F32)
    act = (g * jax.nn.sigmoid(g) * u).astype(_BF)
    d_wd.wait()
    y = jnp.dot(act, wd_v[...], preferred_element_type=_F32)[0:1, :]
    row = of_v[pl.ds(sel, 1), :] + modr(5) * (y * gate_r)

    base = pl.multiple_of((sel // 16) * 16, 16)
    tile = of_v[pl.ds(base, 16), :]
    rid = base + lax.broadcasted_iota(jnp.int32, (16, _D), 0)
    fix_v[...] = jnp.where(rid == sel, row, tile).astype(_BF)

    pltpu.make_async_copy(out_v, out_hbm, sems.at[_SEM_OUT]).wait()
    d_fix = cp(fix_v, out_hbm.at[pl.ds(base, 16)], _SEM_FIX)
    d_fix.start()
    d_fix.wait()


@jax.jit
def pallas_adaLN_cond__sliding_block_cached__moe_arch_mod__prompt_kernel(
    A_x: jax.Array,
    A_k_cache: jax.Array,
    A_v_cache: jax.Array,
    A_wq: jax.Array,
    A_wo: jax.Array,
    B_x: jax.Array,
    B_w_r: jax.Array,
    B_w_gate: jax.Array,
    B_w_up: jax.Array,
    B_w_down: jax.Array,
    c: jax.Array,
    w_mod: jax.Array,
):
    del B_x
    x = A_x.reshape(_S, _D)
    k = A_k_cache.reshape(_HKV, _SK, _DH)
    v = A_v_cache.reshape(_HKV, _SK, _DH)
    wr = B_w_r.reshape(1, _D)

    any_spec = pl.BlockSpec(memory_space=pl.ANY)
    out = pl.pallas_call(
        _kernel,
        out_shape=jax.ShapeDtypeStruct((_S, _D), _BF),
        in_specs=[any_spec] * 11,
        out_specs=any_spec,
        scratch_shapes=[
            pltpu.VMEM((_S, _D), _BF),
            pltpu.VMEM((_M // 2, _D), jnp.uint32),
            pltpu.VMEM((_M // 2, _D), jnp.uint32),
            pltpu.VMEM((_HKV, _W, _DH), _BF),
            pltpu.VMEM((_HKV, _DH // 2, _W), jnp.uint32),
            pltpu.VMEM((_HKV, _W, _DH), _BF),
            pltpu.VMEM((_HKV, _W // 2, _DH), jnp.uint32),
            pltpu.VMEM((_NS, _D, _QC), _BF),
            pltpu.VMEM((_NS, _HQ * _DH, _NT), _BF),
            pltpu.VMEM((_D, 6 * _D), _BF),
            pltpu.VMEM((_D, _F), _BF),
            pltpu.VMEM((_D, _F), _BF),
            pltpu.VMEM((_F, _D), _BF),
            pltpu.VMEM((1, _D), _BF),
            pltpu.VMEM((1, _D), _BF),
            pltpu.VMEM((_NS, _M // 2, _QC), jnp.uint32),
            pltpu.VMEM((_NS, _M // 2, _QC), jnp.uint32),
            pltpu.VMEM((_NS, _M, _NT), _F32),
            pltpu.VMEM((_NS, _M, _NT), _F32),
            pltpu.VMEM((_S, _D), _BF),
            pltpu.VMEM((_S, _D), _F32),
            pltpu.VMEM((_S, _D), _F32),
            pltpu.VMEM((6, 8, _D), _F32),
            pltpu.VMEM((8, 128), _F32),
            pltpu.VMEM((8, 128), jnp.int32),
            pltpu.VMEM((16, _D), _BF),
            pltpu.SemaphoreType.DMA((_NSEM,)),
        ],
        compiler_params=pltpu.CompilerParams(vmem_limit_bytes=110 * 1024 * 1024),
    )(x, k, v, A_wq, A_wo, wr, B_w_gate, B_w_up, B_w_down, c, w_mod)
    return out.reshape(1, _S, _D)
```

```python
import functools

import jax
import jax.numpy as jnp
from jax import lax
from jax.experimental import pallas as pl
from jax.experimental.pallas import tpu as pltpu

_S = 2048
_D = 1024
_HQ = 32
_HKV = 4
_DH = 128
_SK = 2048
_W = min(4096, max(256, _SK // 4))
_F = 3584
_EPS = 1e-5

_M = 512
_NB = _S // _M
_HPS = 4
_NS = _HQ // _HPS
_R = _M // _NS
_QC = _HPS * _DH
_NT = _D // _NS
_SPG = _NS // _HKV
_MC = 512
_NMC = 6 * _D // _MC
_NMA = 2 * _D // _MC
assert _NMC - _NMA == _NS

_LOG2E = 1.4426950408889634
_QSCALE = (_DH ** -0.5) * _LOG2E

_BF = jnp.bfloat16
_F32 = jnp.float32

_SEM_C, _SEM_WR, _SEM_K, _SEM_V = 0, 1, 2, 3
_SEM_MODA, _SEM_MODB, _SEM_WO, _SEM_WG, _SEM_WU, _SEM_WD = 4, 5, 6, 7, 8, 9
_SEM_OUT, _SEM_FIX = 10, 11
_SEM_WQ = 12
_SEM_X = _SEM_WQ + _NS
_NSEM = _SEM_X + _NB


def _kernel(x_hbm, k_hbm, v_hbm, wq_hbm, wo_hbm, wr_hbm, wg_hbm, wu_hbm, wd_hbm, c_hbm, wmod_hbm,
            out_hbm,
            x_v, h_a, h_b, k_v, kT_v, v_v, vv_v, wq_v, wo_v, wmod_v, wg_v, wu_v, wd_v, c_v, wr_v,
            o_a, o_b, a_a, a_b, out_v, h2_v, of_v, mod_v, modq_v, best_v, bidx_v, fix_v, sems):
    h_buf, o_buf, a_buf = (h_a, h_b), (o_a, o_b), (a_a, a_b)

    def cp(src, dst, slot):
        return pltpu.make_async_copy(src, dst, sems.at[slot])

    d_c = cp(c_hbm, c_v, _SEM_C)

    def d_mod(i):
        return cp(wmod_hbm.at[:, pl.ds(i * _MC, _MC)], wmod_v.at[i],
                  _SEM_MODA if i < _NMA else _SEM_MODB)

    d_k = cp(k_hbm.at[:, pl.ds(_SK - _W, _W), :], k_v, _SEM_K)
    d_v = cp(v_hbm.at[:, pl.ds(_SK - _W, _W), :], v_v, _SEM_V)

    def d_wq(j):
        return cp(wq_hbm.at[:, pl.ds(pl.multiple_of(j * _QC, _QC), _QC)], wq_v.at[j], _SEM_WQ + j)

    def d_x(b):
        return cp(x_hbm.at[pl.ds(b * _M, _M)], x_v.at[pl.ds(b * _M, _M)], _SEM_X + b)

    d_wr = cp(wr_hbm, wr_v, _SEM_WR)
    d_wg = cp(wg_hbm, wg_v, _SEM_WG)
    d_wu = cp(wu_hbm, wu_v, _SEM_WU)
    d_wd = cp(wd_hbm, wd_v, _SEM_WD)

    d_c.start()
    d_x(0).start()
    for i in range(_NMA):
        d_mod(i).start()
    d_wq(0).start()
    d_k.start()
    d_v.start()
    d_x(1).start()
    for j in range(1, _NS):
        d_wq(j).start()
    for j in range(_NS):
        cp(wo_hbm.at[:, pl.ds(j * _NT, _NT)], wo_v.at[j], _SEM_WO).start()
    for b in range(2, _NB):
        d_x(b).start()
    d_wr.start()
    for i in range(_NMA, _NMC):
        d_mod(i).start()
    d_wg.start()
    d_wu.start()
    d_wd.start()

    def mod_chunk(i):
        cf = c_v[...].astype(_F32)
        sc = jnp.broadcast_to((cf * jax.nn.sigmoid(cf)).astype(_BF), (16, _D))
        m = jnp.dot(sc, wmod_v[i], preferred_element_type=_F32)
        mod_v[i] = m[0:8, :]

    def modr(i):
        n = _D // _MC
        return jnp.concatenate([mod_v[n * i + u, 0:1, :] for u in range(n)], axis=1)

    def pack(xf):
        return pltpu.bitcast(xf.astype(_BF), jnp.uint32)

    def unpack(w):
        return pltpu.bitcast(w, _BF)

    def ln(xf):
        mu = jnp.mean(xf, axis=1, keepdims=True)
        d = xf - mu
        var = jnp.mean(d * d, axis=1, keepdims=True)
        return d * lax.rsqrt(var + _EPS)

    def ln1_slice(b, i):
        rows = pl.ds(pl.multiple_of(b * _M + i * _R, _R), _R)
        y = ln(x_v[rows, :].astype(_F32))
        h = y * modq_v[1:2, :] + modq_v[0:1, :]
        h_buf[b % 2][pl.ds(pl.multiple_of(i * (_R // 2), _R // 2), _R // 2), :] = pack(h)

    def qproj_head(b, j, hh):
        q = jnp.dot(unpack(h_buf[b % 2][...]), wq_v[j, :, pl.ds(hh * _DH, _DH)],
                    preferred_element_type=_F32)
        return q.astype(_BF)

    def scores(j, q):
        return jnp.dot(q, unpack(kT_v[j // _SPG]), preferred_element_type=_F32)

    def softmax_pv(b, j, hh, s):
        m = jnp.max(s, axis=1, keepdims=True)
        p = jnp.exp2(s - m)
        l = jnp.sum(p, axis=1, keepdims=True)
        o = jnp.dot(p.astype(_BF), unpack(vv_v[j // _SPG]), preferred_element_type=_F32)
        r = pl.reciprocal(l, approx=True)
        r = r * (2.0 - l * r)
        o_buf[b % 2][j, :, pl.ds(hh * _DH, _DH)] = pack(o * r)

    def oproj_part(b, j, part):
        n = _NS // _HPS
        lhs = jnp.concatenate([unpack(o_buf[b % 2][part * n + jj]) for jj in range(n)], axis=1)
        return jnp.dot(lhs, wo_v[j, pl.ds(part * n * _QC, n * _QC), :], preferred_element_type=_F32)

    def epilogue(b, i):
        lrows = pl.ds(pl.multiple_of(i * _R, _R), _R)
        row0 = pl.multiple_of(b * _M + i * _R, _R)
        rows = pl.ds(row0, _R)
        a = jnp.concatenate([a_buf[b % 2][jj, lrows, :] for jj in range(_NS)], axis=1)
        x1 = x_v[rows, :].astype(_F32) + modr(2) * a
        h2 = ln(x1) * (1.0 + modr(4)) + modr(3)
        o = x1 + modr(5) * h2
        out_v[rows, :] = o.astype(_BF)
        h2_v[rows, :] = h2
        of_v[rows, :] = o
        r = jnp.sum(h2 * wr_v[...].astype(_F32), axis=1, keepdims=True)
        r = jnp.broadcast_to(r, (_R, 128))
        ridx = row0 + lax.broadcasted_iota(jnp.int32, (_R, 128), 0)
        bv = best_v[...]
        bi = bidx_v[...]
        for s in range(_R // 8):
            rs = r[s * 8:(s + 1) * 8]
            upd = rs > bv
            bv = jnp.where(upd, rs, bv)
            bi = jnp.where(upd, ridx[s * 8:(s + 1) * 8], bi)
        best_v[...] = bv
        bidx_v[...] = bi

    def block_phase(b):
        do_attn = b < _NB
        do_o = 0 <= b - 1 < _NB
        do_epi = 0 <= b - 2
        do_ln = b + 1 < _NB

        def step(j, carry):
            if b == 0:
                d_wq(j).wait()
            parts = []
            if do_attn:
                q = qproj_head(b, j, 0)
            for hh in range(_HPS):
                if do_o and hh in (0, _HPS - 1):
                    if hh == 0:
                        parts.append(oproj_part(b - 1, j, 0))
                if do_attn:
                    s = scores(j, q)
                    if hh + 1 < _HPS:
                        q = qproj_head(b, j, hh + 1)
                    elif do_o:
                        parts.append(oproj_part(b - 1, j, 1))
                    softmax_pv(b, j, hh, s)
            if b == 1:
                mod_chunk(_NMA + j)
            if do_epi:
                epilogue(b - 2, j)
            if do_ln:
                ln1_slice(b + 1, j)
            if do_o:
                for part in range(len(parts), _HPS):
                    parts.append(oproj_part(b - 1, j, part))
                a_buf[(b - 1) % 2][j] = functools.reduce(lambda u, w: u + w, parts)
            return carry
        lax.fori_loop(0, _NS, step, 0, unroll=(1 if do_attn or do_o else 4))

    def out_copy(b):
        rows = pl.ds(b * _M, _M)
        return cp(out_v.at[rows], out_hbm.at[rows], _SEM_OUT)

    d_c.wait()
    pltpu.make_async_copy(wmod_v.at[pl.ds(0, _NMA)], wmod_v.at[pl.ds(0, _NMA)],
                          sems.at[_SEM_MODA]).wait()
    for i in range(_NMA):
        mod_chunk(i)
    modq_v[0:1, :] = modr(0) * _QSCALE
    modq_v[1:2, :] = (1.0 + modr(1)) * _QSCALE
    d_x(0).wait()
    for i in range(_NS):
        ln1_slice(0, i)
    d_k.wait()
    for g in range(_HKV):
        kT_v[g] = pack(k_v[g].astype(_F32).T)
    d_v.wait()
    for g in range(_HKV):
        vv_v[g] = pltpu.bitcast(v_v[g], jnp.uint32)
    best_v[...] = jnp.full((8, 128), -jnp.inf, _F32)
    bidx_v[...] = jnp.zeros((8, 128), jnp.int32)

    for b in range(_NB + 2):
        if b == 1:
            pltpu.make_async_copy(wo_v, wo_v, sems.at[_SEM_WO]).wait()
            d_wr.wait()
            pltpu.make_async_copy(wmod_v.at[pl.ds(_NMA, _NMC - _NMA)],
                                  wmod_v.at[pl.ds(_NMA, _NMC - _NMA)], sems.at[_SEM_MODB]).wait()
        if b + 1 < _NB:
            d_x(b + 1).wait()
        block_phase(b)
        if b >= 2:
            out_copy(b - 2).start()

    bv = best_v[...]
    bi = bidx_v[...]
    rmax = jnp.max(bv, axis=0, keepdims=True)
    cand = jnp.where(bv == rmax, bi, _S)
    sel = jnp.min(cand)
    sel = jnp.clip(sel, 0, _S - 1)
    gate_r = jax.nn.sigmoid(rmax[:, 0:1])

    xs = h2_v[pl.ds(sel, 1), :].astype(_BF)
    xs = jnp.broadcast_to(xs, (16, _D))
    d_wg.wait()
    d_wu.wait()
    g = jnp.dot(xs, wg_v[...], preferred_element_type=_F32)
    u = jnp.dot(xs, wu_v[...], preferred_element_type=_F32)
    act = (g * jax.nn.sigmoid(g) * u).astype(_BF)
    d_wd.wait()
    y = functools.reduce(lambda u_, w_: u_ + w_, [
        jnp.dot(act[:, i * 512:(i + 1) * 512], wd_v[pl.ds(i * 512, 512), :],
                preferred_element_type=_F32) for i in range(_F // 512)])[0:1, :]
    row = of_v[pl.ds(sel, 1), :] + modr(5) * (y * gate_r)

    base = pl.multiple_of((sel // 16) * 16, 16)
    tile = of_v[pl.ds(base, 16), :]
    rid = base + lax.broadcasted_iota(jnp.int32, (16, _D), 0)
    fix_v[...] = jnp.where(rid == sel, row, tile).astype(_BF)

    pltpu.make_async_copy(out_v, out_hbm, sems.at[_SEM_OUT]).wait()
    d_fix = cp(fix_v, out_hbm.at[pl.ds(base, 16)], _SEM_FIX)
    d_fix.start()
    d_fix.wait()


@jax.jit
def pallas_adaLN_cond__sliding_block_cached__moe_arch_mod__prompt_kernel(
    A_x: jax.Array,
    A_k_cache: jax.Array,
    A_v_cache: jax.Array,
    A_wq: jax.Array,
    A_wo: jax.Array,
    B_x: jax.Array,
    B_w_r: jax.Array,
    B_w_gate: jax.Array,
    B_w_up: jax.Array,
    B_w_down: jax.Array,
    c: jax.Array,
    w_mod: jax.Array,
):
    del B_x
    x = A_x.reshape(_S, _D)
    k = A_k_cache.reshape(_HKV, _SK, _DH)
    v = A_v_cache.reshape(_HKV, _SK, _DH)
    wr = B_w_r.reshape(1, _D)

    any_spec = pl.BlockSpec(memory_space=pl.ANY)
    out = pl.pallas_call(
        _kernel,
        out_shape=jax.ShapeDtypeStruct((_S, _D), _BF),
        in_specs=[any_spec] * 11,
        out_specs=any_spec,
        scratch_shapes=[
            pltpu.VMEM((_S, _D), _BF),
            pltpu.VMEM((_M // 2, _D), jnp.uint32),
            pltpu.VMEM((_M // 2, _D), jnp.uint32),
            pltpu.VMEM((_HKV, _W, _DH), _BF),
            pltpu.VMEM((_HKV, _DH // 2, _W), jnp.uint32),
            pltpu.VMEM((_HKV, _W, _DH), _BF),
            pltpu.VMEM((_HKV, _W // 2, _DH), jnp.uint32),
            pltpu.VMEM((_NS, _D, _QC), _BF),
            pltpu.VMEM((_NS, _HQ * _DH, _NT), _BF),
            pltpu.VMEM((_NMC, _D, _MC), _BF),
            pltpu.VMEM((_D, _F), _BF),
            pltpu.VMEM((_D, _F), _BF),
            pltpu.VMEM((_F, _D), _BF),
            pltpu.VMEM((1, _D), _BF),
            pltpu.VMEM((1, _D), _BF),
            pltpu.VMEM((_NS, _M // 2, _QC), jnp.uint32),
            pltpu.VMEM((_NS, _M // 2, _QC), jnp.uint32),
            pltpu.VMEM((_NS, _M, _NT), _F32),
            pltpu.VMEM((_NS, _M, _NT), _F32),
            pltpu.VMEM((_S, _D), _BF),
            pltpu.VMEM((_S, _D), _F32),
            pltpu.VMEM((_S, _D), _F32),
            pltpu.VMEM((_NMC, 8, _MC), _F32),
            pltpu.VMEM((2, _D), _F32),
            pltpu.VMEM((8, 128), _F32),
            pltpu.VMEM((8, 128), jnp.int32),
            pltpu.VMEM((16, _D), _BF),
            pltpu.SemaphoreType.DMA((_NSEM,)),
        ],
        compiler_params=pltpu.CompilerParams(vmem_limit_bytes=110 * 1024 * 1024),
    )(x, k, v, A_wq, A_wo, wr, B_w_gate, B_w_up, B_w_down, c, w_mod)
    return out.reshape(1, _S, _D)
```

```python
import functools

import jax
import jax.numpy as jnp
from jax import lax
from jax.experimental import pallas as pl
from jax.experimental.pallas import tpu as pltpu

_S = 2048
_D = 1024
_HQ = 32
_HKV = 4
_DH = 128
_SK = 2048
_W = min(4096, max(256, _SK // 4))
_F = 3584
_EPS = 1e-5

_M = 512
_NB = _S // _M
_HPS = 4
_NS = _HQ // _HPS
_R = _M // _NS
_QC = _HPS * _DH
_NT = _D // _NS
_SPG = _NS // _HKV
_MC = 512
_NMC = 6 * _D // _MC
_NMA = 2 * _D // _MC
assert _NMC - _NMA == _NS

_LOG2E = 1.4426950408889634
_QSCALE = (_DH ** -0.5) * _LOG2E

_BF = jnp.bfloat16
_F32 = jnp.float32

_SEM_C, _SEM_WR, _SEM_MODB, _SEM_WO, _SEM_WG, _SEM_WU, _SEM_WD = 0, 1, 2, 3, 4, 5, 6
_SEM_OUT, _SEM_FIX = 7, 8
_SEM_WQ = 9
_SEM_X = _SEM_WQ + _NS
_SEM_X1 = _SEM_X + _NB
_SEM_K = _SEM_X1 + _NS
_SEM_V = _SEM_K + _HKV
_SEM_MODA = _SEM_V + _HKV
_NSEM = _SEM_MODA + _NMA


def _kernel(x_hbm, k_hbm, v_hbm, wq_hbm, wo_hbm, wr_hbm, wg_hbm, wu_hbm, wd_hbm, c_hbm, wmod_hbm,
            out_hbm,
            x_v, h_a, h_b, k_v, v_v, wq_v, wo_v, wmod_v, wg_v, wu_v, wd_v, c_v, wr_v, wrf_v,
            o_a, o_b, a_a, a_b, out_v, h2_v, of_v, mod_v, modq_v, best_v, bidx_v, fix_v, sems):
    h_buf, o_buf, a_buf = (h_a, h_b), (o_a, o_b), (a_a, a_b)

    def cp(src, dst, slot):
        return pltpu.make_async_copy(src, dst, sems.at[slot])

    d_c = cp(c_hbm, c_v, _SEM_C)

    def d_mod(i):
        return cp(wmod_hbm.at[:, pl.ds(i * _MC, _MC)], wmod_v.at[i],
                  _SEM_MODA + i if i < _NMA else _SEM_MODB)

    def d_k(g):
        return cp(k_hbm.at[g, pl.ds(_SK - _W, _W), :], k_v.at[g], _SEM_K + g)

    def d_v(g):
        return cp(v_hbm.at[g, pl.ds(_SK - _W, _W), :], v_v.at[g], _SEM_V + g)

    def d_x1(i):
        rows = pl.ds(pl.multiple_of(_M + i * _R, _R), _R)
        return cp(x_hbm.at[rows], x_v.at[rows], _SEM_X1 + i)

    def d_wq(j):
        return cp(wq_hbm.at[:, pl.ds(pl.multiple_of(j * _QC, _QC), _QC)], wq_v.at[j], _SEM_WQ + j)

    def d_x(b):
        return cp(x_hbm.at[pl.ds(b * _M, _M)], x_v.at[pl.ds(b * _M, _M)], _SEM_X + b)

    d_wr = cp(wr_hbm, wr_v, _SEM_WR)
    d_wg = cp(wg_hbm, wg_v, _SEM_WG)
    d_wu = cp(wu_hbm, wu_v, _SEM_WU)
    d_wd = cp(wd_hbm, wd_v, _SEM_WD)

    d_c.start()
    for i in range(_NMA):
        d_mod(i).start()
    d_x(0).start()
    for j in range(_NS):
        if j % _SPG == 0:
            d_k(j // _SPG).start()
            d_v(j // _SPG).start()
        d_wq(j).start()
        d_x1(j).start()
    for j in range(_NS):
        cp(wo_hbm.at[:, pl.ds(j * _NT, _NT)], wo_v.at[j], _SEM_WO).start()
    for b in range(2, _NB):
        d_x(b).start()
    d_wr.start()
    for i in range(_NMA, _NMC):
        d_mod(i).start()
    d_wg.start()
    d_wu.start()
    d_wd.start()

    def mod_chunk(i):
        cf = c_v[...].astype(_F32)
        sc = jnp.broadcast_to((cf * jax.nn.sigmoid(cf)).astype(_BF), (16, _D))
        m = jnp.dot(sc, wmod_v[i], preferred_element_type=_F32)
        mod_v[i] = m[0:8, :]

    def modr(i):
        n = _D // _MC
        return jnp.concatenate([mod_v[n * i + u, 0:1, :] for u in range(n)], axis=1)

    def pack(xf):
        return pltpu.bitcast(xf.astype(_BF), jnp.uint32)

    def unpack(w):
        return pltpu.bitcast(w, _BF)

    def ln(xf):
        mu = jnp.mean(xf, axis=1, keepdims=True)
        d = xf - mu
        var = jnp.mean(d * d, axis=1, keepdims=True)
        return d * lax.rsqrt(var + _EPS)

    def ln1_slice(b, i):
        rows = pl.ds(pl.multiple_of(b * _M + i * _R, _R), _R)
        y = ln(x_v[rows, :].astype(_F32))
        h = y * modq_v[1:2, :] + modq_v[0:1, :]
        h_buf[b % 2][pl.ds(pl.multiple_of(i * (_R // 2), _R // 2), _R // 2), :] = pack(h)

    def qproj_head(b, j, hh):
        q = jnp.dot(unpack(h_buf[b % 2][...]), wq_v[j, :, pl.ds(hh * _DH, _DH)],
                    preferred_element_type=_F32)
        return q.astype(_BF)

    def scores(j, q):
        return lax.dot_general(q, k_v[j // _SPG], (((1,), (1,)), ((), ())),
                               preferred_element_type=_F32)

    def softmax_pv(b, j, hh, s):
        m = jnp.max(s, axis=1, keepdims=True)
        p = jnp.exp2(s - m)
        l = jnp.sum(p, axis=1, keepdims=True)
        o = jnp.dot(p.astype(_BF), v_v[j // _SPG], preferred_element_type=_F32)
        r = pl.reciprocal(l, approx=True)
        r = r * (2.0 - l * r)
        o_buf[b % 2][j, :, pl.ds(hh * _DH, _DH)] = pack(o * r)

    def oproj_part(b, j, part):
        n = _NS // _HPS
        lhs = jnp.concatenate([unpack(o_buf[b % 2][part * n + jj]) for jj in range(n)], axis=1)
        return jnp.dot(lhs, wo_v[j, pl.ds(part * n * _QC, n * _QC), :], preferred_element_type=_F32)

    def epilogue(b, i):
        lrows = pl.ds(pl.multiple_of(i * _R, _R), _R)
        row0 = pl.multiple_of(b * _M + i * _R, _R)
        rows = pl.ds(row0, _R)
        a = jnp.concatenate([a_buf[b % 2][jj, lrows, :] for jj in range(_NS)], axis=1)
        x1 = x_v[rows, :].astype(_F32) + modr(2) * a
        h2 = ln(x1) * (1.0 + modr(4)) + modr(3)
        o = x1 + modr(5) * h2
        out_v[rows, :] = o.astype(_BF)
        h2_v[rows, :] = h2
        of_v[rows, :] = o
        r = jnp.sum(h2 * wrf_v[...], axis=1, keepdims=True)
        r = jnp.broadcast_to(r, (_R, 128))
        ridx = row0 + lax.broadcasted_iota(jnp.int32, (_R, 128), 0)
        bv = best_v[...]
        bi = bidx_v[...]
        for s in range(_R // 8):
            rs = r[s * 8:(s + 1) * 8]
            upd = rs > bv
            bv = jnp.where(upd, rs, bv)
            bi = jnp.where(upd, ridx[s * 8:(s + 1) * 8], bi)
        best_v[...] = bv
        bidx_v[...] = bi

    def block_phase(b):
        do_attn = b < _NB
        do_o = 0 <= b - 1 < _NB
        do_epi = 0 <= b - 2
        do_ln = b + 1 < _NB

        def step(j, carry):
            if b == 0:
                @pl.when(j % _SPG == 0)
                def _():
                    d_k(j // _SPG).wait()
                    d_v(j // _SPG).wait()
                d_wq(j).wait()
                d_x1(j).wait()
            parts = []
            if do_attn:
                q = qproj_head(b, j, 0)
            for hh in range(_HPS):
                if do_o and hh in (0, _HPS - 1):
                    if hh == 0:
                        parts.append(oproj_part(b - 1, j, 0))
                if do_attn:
                    s = scores(j, q)
                    if hh + 1 < _HPS:
                        q = qproj_head(b, j, hh + 1)
                    elif do_o:
                        parts.append(oproj_part(b - 1, j, 1))
                    softmax_pv(b, j, hh, s)
            if b == 1:
                mod_chunk(_NMA + j)
            if do_epi:
                epilogue(b - 2, j)
            if do_ln:
                ln1_slice(b + 1, j)
            if do_o:
                for part in range(len(parts), _HPS):
                    parts.append(oproj_part(b - 1, j, part))
                a_buf[(b - 1) % 2][j] = functools.reduce(lambda u, w: u + w, parts)
            return carry
        lax.fori_loop(0, _NS, step, 0, unroll=(1 if do_attn or do_o else 4))

    def out_copy(b):
        rows = pl.ds(b * _M, _M)
        return cp(out_v.at[rows], out_hbm.at[rows], _SEM_OUT)

    d_c.wait()
    for i in range(_NMA):
        d_mod(i).wait()
        mod_chunk(i)
    modq_v[0:1, :] = modr(0) * _QSCALE
    modq_v[1:2, :] = (1.0 + modr(1)) * _QSCALE
    d_x(0).wait()
    for i in range(_NS):
        ln1_slice(0, i)
    best_v[...] = jnp.full((8, 128), -jnp.inf, _F32)
    bidx_v[...] = jnp.zeros((8, 128), jnp.int32)

    for b in range(_NB + 2):
        if b == 1:
            pltpu.make_async_copy(wo_v, wo_v, sems.at[_SEM_WO]).wait()
            d_wr.wait()
            wrf_v[...] = wr_v[...].astype(_F32).reshape(1, _D)
            pltpu.make_async_copy(wmod_v.at[pl.ds(_NMA, _NMC - _NMA)],
                                  wmod_v.at[pl.ds(_NMA, _NMC - _NMA)], sems.at[_SEM_MODB]).wait()
        if 2 <= b + 1 < _NB:
            d_x(b + 1).wait()
        block_phase(b)
        if b >= 2:
            out_copy(b - 2).start()

    bv = best_v[...]
    bi = bidx_v[...]
    rmax = jnp.max(bv, axis=0, keepdims=True)
    cand = jnp.where(bv == rmax, bi, _S)
    sel = jnp.min(cand)
    sel = jnp.clip(sel, 0, _S - 1)
    gate_r = jax.nn.sigmoid(rmax[:, 0:1])

    xs = h2_v[pl.ds(sel, 1), :].astype(_BF)
    xs = jnp.broadcast_to(xs, (16, _D))
    d_wg.wait()
    d_wu.wait()
    g = jnp.dot(xs, wg_v[...], preferred_element_type=_F32)
    u = jnp.dot(xs, wu_v[...], preferred_element_type=_F32)
    act = (g * jax.nn.sigmoid(g) * u).astype(_BF)
    d_wd.wait()
    y = functools.reduce(lambda u_, w_: u_ + w_, [
        jnp.dot(act[:, i * 512:(i + 1) * 512], wd_v[pl.ds(i * 512, 512), :],
                preferred_element_type=_F32) for i in range(_F // 512)])[0:1, :]
    row = of_v[pl.ds(sel, 1), :] + modr(5) * (y * gate_r)

    base = pl.multiple_of((sel // 16) * 16, 16)
    tile = of_v[pl.ds(base, 16), :]
    rid = base + lax.broadcasted_iota(jnp.int32, (16, _D), 0)
    fix_v[...] = jnp.where(rid == sel, row, tile).astype(_BF)

    pltpu.make_async_copy(out_v, out_hbm, sems.at[_SEM_OUT]).wait()
    d_fix = cp(fix_v, out_hbm.at[pl.ds(base, 16)], _SEM_FIX)
    d_fix.start()
    d_fix.wait()


@jax.jit
def pallas_adaLN_cond__sliding_block_cached__moe_arch_mod__prompt_kernel(
    A_x: jax.Array,
    A_k_cache: jax.Array,
    A_v_cache: jax.Array,
    A_wq: jax.Array,
    A_wo: jax.Array,
    B_x: jax.Array,
    B_w_r: jax.Array,
    B_w_gate: jax.Array,
    B_w_up: jax.Array,
    B_w_down: jax.Array,
    c: jax.Array,
    w_mod: jax.Array,
):
    del B_x
    x = A_x.reshape(_S, _D)
    k = A_k_cache.reshape(_HKV, _SK, _DH)
    v = A_v_cache.reshape(_HKV, _SK, _DH)

    any_spec = pl.BlockSpec(memory_space=pl.ANY)
    out = pl.pallas_call(
        _kernel,
        out_shape=jax.ShapeDtypeStruct((_S, _D), _BF),
        in_specs=[any_spec] * 11,
        out_specs=any_spec,
        scratch_shapes=[
            pltpu.VMEM((_S, _D), _BF),
            pltpu.VMEM((_M // 2, _D), jnp.uint32),
            pltpu.VMEM((_M // 2, _D), jnp.uint32),
            pltpu.VMEM((_HKV, _W, _DH), _BF),
            pltpu.VMEM((_HKV, _W, _DH), _BF),
            pltpu.VMEM((_NS, _D, _QC), _BF),
            pltpu.VMEM((_NS, _HQ * _DH, _NT), _BF),
            pltpu.VMEM((_NMC, _D, _MC), _BF),
            pltpu.VMEM((_D, _F), _BF),
            pltpu.VMEM((_D, _F), _BF),
            pltpu.VMEM((_F, _D), _BF),
            pltpu.VMEM((1, _D), _BF),
            pltpu.VMEM((_D,), _BF),
            pltpu.VMEM((1, _D), _F32),
            pltpu.VMEM((_NS, _M // 2, _QC), jnp.uint32),
            pltpu.VMEM((_NS, _M // 2, _QC), jnp.uint32),
            pltpu.VMEM((_NS, _M, _NT), _F32),
            pltpu.VMEM((_NS, _M, _NT), _F32),
            pltpu.VMEM((_S, _D), _BF),
            pltpu.VMEM((_S, _D), _F32),
            pltpu.VMEM((_S, _D), _F32),
            pltpu.VMEM((_NMC, 8, _MC), _F32),
            pltpu.VMEM((2, _D), _F32),
            pltpu.VMEM((8, 128), _F32),
            pltpu.VMEM((8, 128), jnp.int32),
            pltpu.VMEM((16, _D), _BF),
            pltpu.SemaphoreType.DMA((_NSEM,)),
        ],
        compiler_params=pltpu.CompilerParams(vmem_limit_bytes=110 * 1024 * 1024),
    )(x, k, v, A_wq, A_wo, B_w_r, B_w_gate, B_w_up, B_w_down, c, w_mod)
    return out.reshape(1, _S, _D)
```

```python
import functools

import jax
import jax.numpy as jnp
from jax import lax
from jax.experimental import pallas as pl
from jax.experimental.pallas import tpu as pltpu

_S = 2048
_D = 1024
_HQ = 32
_HKV = 4
_DH = 128
_SK = 2048
_W = min(4096, max(256, _SK // 4))
_F = 3584
_EPS = 1e-5

_M = 512
_NB = _S // _M
_HPS = 4
_NS = _HQ // _HPS
_R = _M // _NS
_QC = _HPS * _DH
_NT = _D // _NS
_SPG = _NS // _HKV
_TIE_Q = 1
_TIE_O = 2
_MC = 512
_NMC = 6 * _D // _MC
_NMA = 2 * _D // _MC
assert _NMC - _NMA == _NS

_LOG2E = 1.4426950408889634
_QSCALE = (_DH ** -0.5) * _LOG2E

_BF = jnp.bfloat16
_F32 = jnp.float32

_SEM_C, _SEM_WR, _SEM_MODB, _SEM_WO, _SEM_WG, _SEM_WU, _SEM_WD = 0, 1, 2, 3, 4, 5, 6
_SEM_OUT, _SEM_FIX = 7, 8
_SEM_WQ = 9
_SEM_X = _SEM_WQ + _NS
_SEM_X1 = _SEM_X + _NB
_SEM_K = _SEM_X1 + _NS
_SEM_V = _SEM_K + _HKV
_SEM_MODA = _SEM_V + _HKV
_NSEM = _SEM_MODA + _NMA


def _kernel(x_hbm, k_hbm, v_hbm, wq_hbm, wo_hbm, wr_hbm, wg_hbm, wu_hbm, wd_hbm, c_hbm, wmod_hbm,
            out_hbm,
            x_v, h_a, h_b, k_v, v_v, wq_v, wo_v, wmod_v, wg_v, wu_v, wd_v, c_v, wr_v, wrf_v,
            o_a, o_b, a_a, a_b, out_v, h2_v, of_v, mod_v, modq_v, best_v, bidx_v, fix_v, sems):
    h_buf, o_buf, a_buf = (h_a, h_b), (o_a, o_b), (a_a, a_b)

    def cp(src, dst, slot):
        return pltpu.make_async_copy(src, dst, sems.at[slot])

    d_c = cp(c_hbm, c_v, _SEM_C)

    def d_mod(i):
        return cp(wmod_hbm.at[:, pl.ds(i * _MC, _MC)], wmod_v.at[i],
                  _SEM_MODA + i if i < _NMA else _SEM_MODB)

    def d_k(g):
        return cp(k_hbm.at[g, pl.ds(_SK - _W, _W), :], k_v.at[g], _SEM_K + g)

    def d_v(g):
        return cp(v_hbm.at[g, pl.ds(_SK - _W, _W), :], v_v.at[g], _SEM_V + g)

    def d_x1(i):
        rows = pl.ds(pl.multiple_of(_M + i * _R, _R), _R)
        return cp(x_hbm.at[rows], x_v.at[rows], _SEM_X1 + i)

    def d_wq(j):
        return cp(wq_hbm.at[:, pl.ds(pl.multiple_of(j * _QC, _QC), _QC)], wq_v.at[j], _SEM_WQ + j)

    def d_x(b):
        return cp(x_hbm.at[pl.ds(b * _M, _M)], x_v.at[pl.ds(b * _M, _M)], _SEM_X + b)

    d_wr = cp(wr_hbm, wr_v, _SEM_WR)
    d_wg = cp(wg_hbm, wg_v, _SEM_WG)
    d_wu = cp(wu_hbm, wu_v, _SEM_WU)
    d_wd = cp(wd_hbm, wd_v, _SEM_WD)

    d_c.start()
    for i in range(_NMA):
        d_mod(i).start()
    d_x(0).start()
    for j in range(_NS):
        if j % _SPG == 0:
            d_k(j // _SPG).start()
            d_v(j // _SPG).start()
        d_wq(j).start()
        d_x1(j).start()
    for j in range(_NS):
        cp(wo_hbm.at[:, pl.ds(j * _NT, _NT)], wo_v.at[j], _SEM_WO).start()
    for b in range(2, _NB):
        d_x(b).start()
    d_wr.start()
    for i in range(_NMA, _NMC):
        d_mod(i).start()
    d_wg.start()
    d_wu.start()
    d_wd.start()

    def mod_chunk(i):
        cf = c_v[...].astype(_F32)
        sc = jnp.broadcast_to((cf * jax.nn.sigmoid(cf)).astype(_BF), (16, _D))
        m = jnp.dot(sc, wmod_v[i], preferred_element_type=_F32)
        mod_v[i] = m[0:8, :]

    def modr(i):
        n = _D // _MC
        return jnp.concatenate([mod_v[n * i + u, 0:1, :] for u in range(n)], axis=1)

    def pack(xf):
        return pltpu.bitcast(xf.astype(_BF), jnp.uint32)

    def unpack(w):
        return pltpu.bitcast(w, _BF)

    def ln(xf):
        mu = jnp.mean(xf, axis=1, keepdims=True)
        d = xf - mu
        var = jnp.mean(d * d, axis=1, keepdims=True)
        return d * lax.rsqrt(var + _EPS)

    def ln1_slice(b, i):
        rows = pl.ds(pl.multiple_of(b * _M + i * _R, _R), _R)
        y = ln(x_v[rows, :].astype(_F32))
        h = y * modq_v[1:2, :] + modq_v[0:1, :]
        h_buf[b % 2][pl.ds(pl.multiple_of(i * (_R // 2), _R // 2), _R // 2), :] = pack(h)

    def tie(w, token):
        if token is None:
            return w
        return jnp.concatenate([w[0:8, 0:128] | token, w[0:8, 128:]], axis=1) if w.shape[0] == 8 else \
            jnp.concatenate([jnp.concatenate([w[0:8, 0:128] | token, w[0:8, 128:]], axis=1), w[8:]], axis=0)

    def qproj_head(b, j, hh, token=None):
        q = jnp.dot(unpack(tie(h_buf[b % 2][...], token)), wq_v[j, :, pl.ds(hh * _DH, _DH)],
                    preferred_element_type=_F32)
        return q.astype(_BF)

    def scores(j, q):
        return lax.dot_general(q, k_v[j // _SPG], (((1,), (1,)), ((), ())),
                               preferred_element_type=_F32)

    def softmax_pv(b, j, hh, s):
        m = jnp.max(s, axis=1, keepdims=True)
        p = jnp.exp2(s - m)
        l = jnp.sum(p, axis=1, keepdims=True)
        o = jnp.dot(p.astype(_BF), v_v[j // _SPG], preferred_element_type=_F32)
        r = pl.reciprocal(l, approx=True)
        r = r * (2.0 - l * r)
        o_buf[b % 2][j, :, pl.ds(hh * _DH, _DH)] = pack(o * r)

    def oproj_part(b, j, part, token=None):
        n = _NS // _HPS
        lhs = jnp.concatenate([unpack(tie(o_buf[b % 2][part * n + jj], token if jj == 0 else None))
                               for jj in range(n)], axis=1)
        return jnp.dot(lhs, wo_v[j, pl.ds(part * n * _QC, n * _QC), :], preferred_element_type=_F32)

    def epilogue(b, i):
        lrows = pl.ds(pl.multiple_of(i * _R, _R), _R)
        row0 = pl.multiple_of(b * _M + i * _R, _R)
        rows = pl.ds(row0, _R)
        a = jnp.concatenate([a_buf[b % 2][jj, lrows, :] for jj in range(_NS)], axis=1)
        x1 = x_v[rows, :].astype(_F32) + modr(2) * a
        h2 = ln(x1) * (1.0 + modr(4)) + modr(3)
        o = x1 + modr(5) * h2
        out_v[rows, :] = o.astype(_BF)
        h2_v[rows, :] = h2
        of_v[rows, :] = o
        r = jnp.sum(h2 * wrf_v[...], axis=1, keepdims=True)
        r = jnp.broadcast_to(r, (_R, 128))
        ridx = row0 + lax.broadcasted_iota(jnp.int32, (_R, 128), 0)
        bv = best_v[...]
        bi = bidx_v[...]
        for s in range(_R // 8):
            rs = r[s * 8:(s + 1) * 8]
            upd = rs > bv
            bv = jnp.where(upd, rs, bv)
            bi = jnp.where(upd, ridx[s * 8:(s + 1) * 8], bi)
        best_v[...] = bv
        bidx_v[...] = bi
        return lax.shift_right_logical(bi, 31).astype(jnp.uint32)

    def block_phase(b):
        do_attn = b < _NB
        do_o = 0 <= b - 1 < _NB
        do_epi = 0 <= b - 2
        do_ln = b + 1 < _NB

        def step(j, carry):
            token = None
            if do_epi:
                token = epilogue(b - 2, j)
            if b == 0:
                @pl.when(j % _SPG == 0)
                def _():
                    d_k(j // _SPG).wait()
                    d_v(j // _SPG).wait()
                d_wq(j).wait()
                d_x1(j).wait()
            parts = []
            if do_attn:
                q = qproj_head(b, j, 0)
            for hh in range(_HPS):
                if do_o and hh == 0:
                    parts.append(oproj_part(b - 1, j, 0))
                if do_attn:
                    s = scores(j, q)
                    if hh + 1 < _HPS:
                        q = qproj_head(b, j, hh + 1, token if hh + 1 == _TIE_Q else None)
                    elif do_o:
                        parts.append(oproj_part(b - 1, j, 1, token if _TIE_Q is None else None))
                    softmax_pv(b, j, hh, s)
            if b == 1:
                mod_chunk(_NMA + j)
            if do_ln:
                ln1_slice(b + 1, j)
            if do_o:
                for part in range(len(parts), _HPS):
                    parts.append(oproj_part(b - 1, j, part,
                                            token if not do_attn and part == _TIE_O else None))
                a_buf[(b - 1) % 2][j] = functools.reduce(lambda u, w: u + w, parts)
            return carry
        lax.fori_loop(0, _NS, step, 0, unroll=(1 if do_attn or do_o else 4))

    def out_copy(b):
        rows = pl.ds(b * _M, _M)
        return cp(out_v.at[rows], out_hbm.at[rows], _SEM_OUT)

    d_c.wait()
    for i in range(_NMA):
        d_mod(i).wait()
        mod_chunk(i)
    modq_v[0:1, :] = modr(0) * _QSCALE
    modq_v[1:2, :] = (1.0 + modr(1)) * _QSCALE
    d_x(0).wait()
    for i in range(_NS):
        ln1_slice(0, i)
    best_v[...] = jnp.full((8, 128), -jnp.inf, _F32)
    bidx_v[...] = jnp.zeros((8, 128), jnp.int32)

    for b in range(_NB + 2):
        if b == 1:
            pltpu.make_async_copy(wo_v, wo_v, sems.at[_SEM_WO]).wait()
            d_wr.wait()
            wrf_v[...] = wr_v[...].astype(_F32).reshape(1, _D)
            pltpu.make_async_copy(wmod_v.at[pl.ds(_NMA, _NMC - _NMA)],
                                  wmod_v.at[pl.ds(_NMA, _NMC - _NMA)], sems.at[_SEM_MODB]).wait()
        if 2 <= b + 1 < _NB:
            d_x(b + 1).wait()
        block_phase(b)
        if b >= 2:
            out_copy(b - 2).start()

    bv = best_v[...]
    bi = bidx_v[...]
    rmax = jnp.max(bv, axis=0, keepdims=True)
    cand = jnp.where(bv == rmax, bi, _S)
    sel = jnp.min(cand)
    sel = jnp.clip(sel, 0, _S - 1)
    gate_r = jax.nn.sigmoid(rmax[:, 0:1])

    xs = h2_v[pl.ds(sel, 1), :].astype(_BF)
    xs = jnp.broadcast_to(xs, (16, _D))
    d_wg.wait()
    d_wu.wait()
    g = jnp.dot(xs, wg_v[...], preferred_element_type=_F32)
    u = jnp.dot(xs, wu_v[...], preferred_element_type=_F32)
    act = (g * jax.nn.sigmoid(g) * u).astype(_BF)
    d_wd.wait()
    y = functools.reduce(lambda u_, w_: u_ + w_, [
        jnp.dot(act[:, i * 512:(i + 1) * 512], wd_v[pl.ds(i * 512, 512), :],
                preferred_element_type=_F32) for i in range(_F // 512)])[0:1, :]
    row = of_v[pl.ds(sel, 1), :] + modr(5) * (y * gate_r)

    base = pl.multiple_of((sel // 16) * 16, 16)
    tile = of_v[pl.ds(base, 16), :]
    rid = base + lax.broadcasted_iota(jnp.int32, (16, _D), 0)
    fix_v[...] = jnp.where(rid == sel, row, tile).astype(_BF)

    pltpu.make_async_copy(out_v, out_hbm, sems.at[_SEM_OUT]).wait()
    d_fix = cp(fix_v, out_hbm.at[pl.ds(base, 16)], _SEM_FIX)
    d_fix.start()
    d_fix.wait()


@jax.jit
def pallas_adaLN_cond__sliding_block_cached__moe_arch_mod__prompt_kernel(
    A_x: jax.Array,
    A_k_cache: jax.Array,
    A_v_cache: jax.Array,
    A_wq: jax.Array,
    A_wo: jax.Array,
    B_x: jax.Array,
    B_w_r: jax.Array,
    B_w_gate: jax.Array,
    B_w_up: jax.Array,
    B_w_down: jax.Array,
    c: jax.Array,
    w_mod: jax.Array,
):
    del B_x
    x = A_x.reshape(_S, _D)
    k = A_k_cache.reshape(_HKV, _SK, _DH)
    v = A_v_cache.reshape(_HKV, _SK, _DH)

    any_spec = pl.BlockSpec(memory_space=pl.ANY)
    out = pl.pallas_call(
        _kernel,
        out_shape=jax.ShapeDtypeStruct((_S, _D), _BF),
        in_specs=[any_spec] * 11,
        out_specs=any_spec,
        scratch_shapes=[
            pltpu.VMEM((_S, _D), _BF),
            pltpu.VMEM((_M // 2, _D), jnp.uint32),
            pltpu.VMEM((_M // 2, _D), jnp.uint32),
            pltpu.VMEM((_HKV, _W, _DH), _BF),
            pltpu.VMEM((_HKV, _W, _DH), _BF),
            pltpu.VMEM((_NS, _D, _QC), _BF),
            pltpu.VMEM((_NS, _HQ * _DH, _NT), _BF),
            pltpu.VMEM((_NMC, _D, _MC), _BF),
            pltpu.VMEM((_D, _F), _BF),
            pltpu.VMEM((_D, _F), _BF),
            pltpu.VMEM((_F, _D), _BF),
            pltpu.VMEM((1, _D), _BF),
            pltpu.VMEM((_D,), _BF),
            pltpu.VMEM((1, _D), _F32),
            pltpu.VMEM((_NS, _M // 2, _QC), jnp.uint32),
            pltpu.VMEM((_NS, _M // 2, _QC), jnp.uint32),
            pltpu.VMEM((_NS, _M, _NT), _F32),
            pltpu.VMEM((_NS, _M, _NT), _F32),
            pltpu.VMEM((_S, _D), _BF),
            pltpu.VMEM((_S, _D), _F32),
            pltpu.VMEM((_S, _D), _F32),
            pltpu.VMEM((_NMC, 8, _MC), _F32),
            pltpu.VMEM((2, _D), _F32),
            pltpu.VMEM((8, 128), _F32),
            pltpu.VMEM((8, 128), jnp.int32),
            pltpu.VMEM((16, _D), _BF),
            pltpu.SemaphoreType.DMA((_NSEM,)),
        ],
        compiler_params=pltpu.CompilerParams(vmem_limit_bytes=110 * 1024 * 1024),
    )(x, k, v, A_wq, A_wo, B_w_r, B_w_gate, B_w_up, B_w_down, c, w_mod)
    return out.reshape(1, _S, _D)
```

```python
import functools

import jax
import jax.numpy as jnp
from jax import lax
from jax.experimental import pallas as pl
from jax.experimental.pallas import tpu as pltpu

_S = 2048
_D = 1024
_HQ = 32
_HKV = 4
_DH = 128
_SK = 2048
_W = min(4096, max(256, _SK // 4))
_F = 3584
_EPS = 1e-5

_M = 512
_NB = _S // _M
_HPS = 4
_NS = _HQ // _HPS
_R = _M // _NS
_QC = _HPS * _DH
_NT = _D // _NS
_SPG = _NS // _HKV
_OW = 512
_NOC = _HQ * _DH // _OW
_HPC = _OW // _DH
_TIE_Q = 1
_TIE_O = 2
_MC = 512
_NMC = 6 * _D // _MC
_NMA = 2 * _D // _MC
assert (_NMC - _NMA) % _NS == 0

_LOG2E = 1.4426950408889634
_QSCALE = (_DH ** -0.5) * _LOG2E

_BF = jnp.bfloat16
_F32 = jnp.float32

_SEM_C, _SEM_WR, _SEM_MODB, _SEM_WO, _SEM_WG, _SEM_WU, _SEM_WD = 0, 1, 2, 3, 4, 5, 6
_SEM_OUT, _SEM_FIX = 7, 8
_SEM_WQ = 9
_SEM_X = _SEM_WQ + _NS
_SEM_X1 = _SEM_X + _NB
_SEM_K = _SEM_X1 + _NS
_SEM_V = _SEM_K + _HKV
_SEM_MODA = _SEM_V + _HKV
_NSEM = _SEM_MODA + _NMA


def _kernel(x_hbm, k_hbm, v_hbm, wq_hbm, wo_hbm, wr_hbm, wg_hbm, wu_hbm, wd_hbm, c_hbm, wmod_hbm,
            out_hbm,
            x_v, h_a, h_b, k_v, v_v, wq_v, wo_v, wmod_v, wg_v, wu_v, wd_v, c_v, wr_v, wrf_v,
            o_a, o_b, a_a, a_b, out_v, h2_v, of_v, mod_v, modq_v, scol_v, best_v, bidx_v, fix_v, sems):
    h_buf, o_buf, a_buf = (h_a, h_b), (o_a, o_b), (a_a, a_b)

    def cp(src, dst, slot):
        return pltpu.make_async_copy(src, dst, sems.at[slot])

    d_c = cp(c_hbm, c_v, _SEM_C)

    def d_mod(i):
        return cp(wmod_hbm.at[:, pl.ds(i * _MC, _MC)], wmod_v.at[i],
                  _SEM_MODA + i if i < _NMA else _SEM_MODB)

    def d_k(g):
        return cp(k_hbm.at[g, pl.ds(_SK - _W, _W), :], k_v.at[g], _SEM_K + g)

    def d_v(g):
        return cp(v_hbm.at[g, pl.ds(_SK - _W, _W), :], v_v.at[g], _SEM_V + g)

    def d_x1(i):
        rows = pl.ds(pl.multiple_of(_M + i * _R, _R), _R)
        return cp(x_hbm.at[rows], x_v.at[rows], _SEM_X1 + i)

    def d_wq(j):
        return cp(wq_hbm.at[:, pl.ds(pl.multiple_of(j * _QC, _QC), _QC)], wq_v.at[j], _SEM_WQ + j)

    def d_x(b):
        return cp(x_hbm.at[pl.ds(b * _M, _M)], x_v.at[pl.ds(b * _M, _M)], _SEM_X + b)

    d_wr = cp(wr_hbm, wr_v, _SEM_WR)
    d_wg = cp(wg_hbm, wg_v, _SEM_WG)
    d_wu = cp(wu_hbm, wu_v, _SEM_WU)
    d_wd = cp(wd_hbm, wd_v, _SEM_WD)

    d_c.start()
    for i in range(_NMA):
        d_mod(i).start()
    d_x(0).start()
    for j in range(_NS):
        if j % _SPG == 0:
            d_k(j // _SPG).start()
            d_v(j // _SPG).start()
        d_wq(j).start()
        d_x1(j).start()
    for j in range(_NS):
        cp(wo_hbm.at[:, pl.ds(j * _NT, _NT)], wo_v.at[j], _SEM_WO).start()
    for b in range(2, _NB):
        d_x(b).start()
    d_wr.start()
    for i in range(_NMA, _NMC):
        d_mod(i).start()
    d_wg.start()
    d_wu.start()
    d_wd.start()

    def mod_chunk(i):
        cf = c_v[...].astype(_F32)
        sc = jnp.broadcast_to((cf * jax.nn.sigmoid(cf)).astype(_BF), (16, _D))
        m = jnp.dot(sc, wmod_v[i], preferred_element_type=_F32)
        mod_v[i] = m[0:8, :]

    def mod_chunk_vpu(i):
        col = scol_v[...]
        outs = []
        for t in range(_MC // 128):
            w = wmod_v[i, :, pl.ds(t * 128, 128)].astype(_F32)
            outs.append(jnp.sum(w * col, axis=0, keepdims=True))
        mod_v[i, 0:1, :] = jnp.concatenate(outs, axis=1)

    def modr(i):
        n = _D // _MC
        return jnp.concatenate([mod_v[n * i + u, 0:1, :] for u in range(n)], axis=1)

    def pack(xf):
        return pltpu.bitcast(xf.astype(_BF), jnp.uint32)

    def unpack(w):
        return pltpu.bitcast(w, _BF)

    def ln(xf):
        mu = jnp.mean(xf, axis=1, keepdims=True)
        d = xf - mu
        var = jnp.mean(d * d, axis=1, keepdims=True)
        return d * lax.rsqrt(var + _EPS)

    def ln1_slice(b, i):
        rows = pl.ds(pl.multiple_of(b * _M + i * _R, _R), _R)
        y = ln(x_v[rows, :].astype(_F32))
        h = y * modq_v[1:2, :] + modq_v[0:1, :]
        h_buf[b % 2][pl.ds(pl.multiple_of(i * (_R // 2), _R // 2), _R // 2), :] = pack(h)

    def tie(w, token):
        if token is None:
            return w
        return jnp.concatenate([w[0:8, 0:128] | token, w[0:8, 128:]], axis=1) if w.shape[0] == 8 else \
            jnp.concatenate([jnp.concatenate([w[0:8, 0:128] | token, w[0:8, 128:]], axis=1), w[8:]], axis=0)

    def qproj_head(b, j, hh, token=None):
        q = jnp.dot(unpack(tie(h_buf[b % 2][...], token)), wq_v[j, :, pl.ds(hh * _DH, _DH)],
                    preferred_element_type=_F32)
        return q.astype(_BF)

    def scores(j, q):
        return lax.dot_general(q, k_v[j // _SPG], (((1,), (1,)), ((), ())),
                               preferred_element_type=_F32)

    def softmax_pv(b, j, hh, s):
        m = jnp.max(s, axis=1, keepdims=True)
        p = jnp.exp2(s - m)
        l = jnp.sum(p, axis=1, keepdims=True)
        o = jnp.dot(p.astype(_BF), v_v[j // _SPG], preferred_element_type=_F32)
        r = pl.reciprocal(l, approx=True)
        r = r * (2.0 - l * r)
        o_buf[b % 2][j * (_HPS // _HPC) + hh // _HPC, :, pl.ds((hh % _HPC) * _DH, _DH)] = pack(o * r)

    def oproj_part(b, j, part, token=None):
        n = _NOC // _HPS
        lhs = jnp.concatenate([unpack(tie(o_buf[b % 2][part * n + jj], token if jj == 0 else None))
                               for jj in range(n)], axis=1)
        return jnp.dot(lhs, wo_v[j, pl.ds(part * n * _OW, n * _OW), :], preferred_element_type=_F32)

    def epilogue(b, i):
        lrows = pl.ds(pl.multiple_of(i * _R, _R), _R)
        row0 = pl.multiple_of(b * _M + i * _R, _R)
        rows = pl.ds(row0, _R)
        a = jnp.concatenate([a_buf[b % 2][jj, lrows, :] for jj in range(_NS)], axis=1)
        x1 = x_v[rows, :].astype(_F32) + modr(2) * a
        h2 = ln(x1) * (1.0 + modr(4)) + modr(3)
        o = x1 + modr(5) * h2
        out_v[rows, :] = o.astype(_BF)
        h2_v[rows, :] = h2
        of_v[rows, :] = o
        r = jnp.sum(h2 * wrf_v[...], axis=1, keepdims=True)
        r = jnp.broadcast_to(r, (_R, 128))
        ridx = row0 + lax.broadcasted_iota(jnp.int32, (_R, 128), 0)
        bv = best_v[...]
        bi = bidx_v[...]
        for s in range(_R // 8):
            rs = r[s * 8:(s + 1) * 8]
            upd = rs > bv
            bv = jnp.where(upd, rs, bv)
            bi = jnp.where(upd, ridx[s * 8:(s + 1) * 8], bi)
        best_v[...] = bv
        bidx_v[...] = bi
        return lax.shift_right_logical(bi, 31).astype(jnp.uint32)

    def block_phase(b):
        do_attn = b < _NB
        do_o = 0 <= b - 1 < _NB
        do_epi = 0 <= b - 2
        do_ln = b + 1 < _NB

        def step(j, carry):
            token = None
            if do_epi:
                token = epilogue(b - 2, j)
            if b == 0:
                @pl.when(j % _SPG == 0)
                def _():
                    d_k(j // _SPG).wait()
                    d_v(j // _SPG).wait()
                d_wq(j).wait()
                d_x1(j).wait()
            parts = []
            if do_attn:
                q = qproj_head(b, j, 0)
            for hh in range(_HPS):
                if do_o and hh == 0:
                    parts.append(oproj_part(b - 1, j, 0))
                if do_attn:
                    s = scores(j, q)
                    if hh + 1 < _HPS:
                        q = qproj_head(b, j, hh + 1, token if hh + 1 == _TIE_Q else None)
                    elif do_o:
                        parts.append(oproj_part(b - 1, j, 1, token if _TIE_Q is None else None))
                    softmax_pv(b, j, hh, s)
            if b == 1:
                for u in range((_NMC - _NMA) // _NS):
                    mod_chunk_vpu(_NMA + j * ((_NMC - _NMA) // _NS) + u)
            if do_ln:
                ln1_slice(b + 1, j)
            if do_o:
                for part in range(len(parts), _HPS):
                    parts.append(oproj_part(b - 1, j, part,
                                            token if not do_attn and part == _TIE_O else None))
                a_buf[(b - 1) % 2][j] = functools.reduce(lambda u, w: u + w, parts)
            return carry
        lax.fori_loop(0, _NS, step, 0, unroll=(1 if do_attn or do_o else _NS // 2))

    def out_copy(b):
        rows = pl.ds(b * _M, _M)
        return cp(out_v.at[rows], out_hbm.at[rows], _SEM_OUT)

    d_c.wait()
    cf = c_v[...].astype(_F32)
    sc = (cf * jax.nn.sigmoid(cf)).astype(_BF).astype(_F32)
    scol_v[...] = jnp.broadcast_to(sc, (128, _D)).T
    for i in range(_NMA):
        d_mod(i).wait()
        mod_chunk(i)
    modq_v[0:1, :] = modr(0) * _QSCALE
    modq_v[1:2, :] = (1.0 + modr(1)) * _QSCALE
    d_x(0).wait()
    for i in range(_NS):
        ln1_slice(0, i)
    best_v[...] = jnp.full((8, 128), -jnp.inf, _F32)
    bidx_v[...] = jnp.zeros((8, 128), jnp.int32)

    for b in range(_NB + 2):
        if b == 1:
            pltpu.make_async_copy(wo_v, wo_v, sems.at[_SEM_WO]).wait()
            d_wr.wait()
            wrf_v[...] = wr_v[...].astype(_F32).reshape(1, _D)
            pltpu.make_async_copy(wmod_v.at[pl.ds(_NMA, _NMC - _NMA)],
                                  wmod_v.at[pl.ds(_NMA, _NMC - _NMA)], sems.at[_SEM_MODB]).wait()
        if 2 <= b + 1 < _NB:
            d_x(b + 1).wait()
        block_phase(b)
        if b >= 2:
            out_copy(b - 2).start()

    bv = best_v[...]
    bi = bidx_v[...]
    rmax = jnp.max(bv, axis=0, keepdims=True)
    cand = jnp.where(bv == rmax, bi, _S)
    sel = jnp.min(cand)
    sel = jnp.clip(sel, 0, _S - 1)
    gate_r = jax.nn.sigmoid(rmax[:, 0:1])

    xs = h2_v[pl.ds(sel, 1), :].astype(_BF)
    xs = jnp.broadcast_to(xs, (16, _D))
    d_wg.wait()
    d_wu.wait()
    g = jnp.dot(xs, wg_v[...], preferred_element_type=_F32)
    u = jnp.dot(xs, wu_v[...], preferred_element_type=_F32)
    act = (g * jax.nn.sigmoid(g) * u).astype(_BF)
    d_wd.wait()
    y = functools.reduce(lambda u_, w_: u_ + w_, [
        jnp.dot(act[:, i * 512:(i + 1) * 512], wd_v[pl.ds(i * 512, 512), :],
                preferred_element_type=_F32) for i in range(_F // 512)])[0:1, :]
    row = of_v[pl.ds(sel, 1), :] + modr(5) * (y * gate_r)

    base = pl.multiple_of((sel // 16) * 16, 16)
    tile = of_v[pl.ds(base, 16), :]
    rid = base + lax.broadcasted_iota(jnp.int32, (16, _D), 0)
    fix_v[...] = jnp.where(rid == sel, row, tile).astype(_BF)

    pltpu.make_async_copy(out_v, out_hbm, sems.at[_SEM_OUT]).wait()
    d_fix = cp(fix_v, out_hbm.at[pl.ds(base, 16)], _SEM_FIX)
    d_fix.start()
    d_fix.wait()


@jax.jit
def pallas_adaLN_cond__sliding_block_cached__moe_arch_mod__prompt_kernel(
    A_x: jax.Array,
    A_k_cache: jax.Array,
    A_v_cache: jax.Array,
    A_wq: jax.Array,
    A_wo: jax.Array,
    B_x: jax.Array,
    B_w_r: jax.Array,
    B_w_gate: jax.Array,
    B_w_up: jax.Array,
    B_w_down: jax.Array,
    c: jax.Array,
    w_mod: jax.Array,
):
    del B_x
    x = A_x.reshape(_S, _D)
    k = A_k_cache.reshape(_HKV, _SK, _DH)
    v = A_v_cache.reshape(_HKV, _SK, _DH)

    any_spec = pl.BlockSpec(memory_space=pl.ANY)
    out = pl.pallas_call(
        _kernel,
        out_shape=jax.ShapeDtypeStruct((_S, _D), _BF),
        in_specs=[any_spec] * 11,
        out_specs=any_spec,
        scratch_shapes=[
            pltpu.VMEM((_S, _D), _BF),
            pltpu.VMEM((_M // 2, _D), jnp.uint32),
            pltpu.VMEM((_M // 2, _D), jnp.uint32),
            pltpu.VMEM((_HKV, _W, _DH), _BF),
            pltpu.VMEM((_HKV, _W, _DH), _BF),
            pltpu.VMEM((_NS, _D, _QC), _BF),
            pltpu.VMEM((_NS, _HQ * _DH, _NT), _BF),
            pltpu.VMEM((_NMC, _D, _MC), _BF),
            pltpu.VMEM((_D, _F), _BF),
            pltpu.VMEM((_D, _F), _BF),
            pltpu.VMEM((_F, _D), _BF),
            pltpu.VMEM((1, _D), _BF),
            pltpu.VMEM((_D,), _BF),
            pltpu.VMEM((1, _D), _F32),
            pltpu.VMEM((_NOC, _M // 2, _OW), jnp.uint32),
            pltpu.VMEM((_NOC, _M // 2, _OW), jnp.uint32),
            pltpu.VMEM((_NS, _M, _NT), _F32),
            pltpu.VMEM((_NS, _M, _NT), _F32),
            pltpu.VMEM((_S, _D), _BF),
            pltpu.VMEM((_S, _D), _F32),
            pltpu.VMEM((_S, _D), _F32),
            pltpu.VMEM((_NMC, 8, _MC), _F32),
            pltpu.VMEM((2, _D), _F32),
            pltpu.VMEM((_D, 128), _F32),
            pltpu.VMEM((8, 128), _F32),
            pltpu.VMEM((8, 128), jnp.int32),
            pltpu.VMEM((16, _D), _BF),
            pltpu.SemaphoreType.DMA((_NSEM,)),
        ],
        compiler_params=pltpu.CompilerParams(vmem_limit_bytes=110 * 1024 * 1024),
    )(x, k, v, A_wq, A_wo, B_w_r, B_w_gate, B_w_up, B_w_down, c, w_mod)
    return out.reshape(1, _S, _D)
```

```python
import functools

import jax
import jax.numpy as jnp
from jax import lax
from jax.experimental import pallas as pl
from jax.experimental.pallas import tpu as pltpu

_S = 2048
_D = 1024
_HQ = 32
_HKV = 4
_DH = 128
_SK = 2048
_W = min(4096, max(256, _SK // 4))
_F = 3584
_EPS = 1e-5

_M = 512
_NB = _S // _M
_HPS = 4
_NS = _HQ // _HPS
_R = _M // _NS
_QC = _HPS * _DH
_NT = _D // _NS
_SPG = _NS // _HKV
_OW = 512
_NOC = _HQ * _DH // _OW
_HPC = _OW // _DH
_TIE_Q = 1
_TIE_D = ((2, 1), (None, 2))
_MC = 512
_NMC = 6 * _D // _MC
_NMA = 2 * _D // _MC
assert (_NMC - _NMA) % _NS == 0

_LOG2E = 1.4426950408889634
_QSCALE = (_DH ** -0.5) * _LOG2E

_BF = jnp.bfloat16
_F32 = jnp.float32

_SEM_C, _SEM_WR, _SEM_MODB, _SEM_WO, _SEM_WG, _SEM_WU, _SEM_WD = 0, 1, 2, 3, 4, 5, 6
_SEM_OUT, _SEM_FIX = 7, 8
_SEM_WQ = 9
_SEM_X = _SEM_WQ + _NS
_SEM_X1 = _SEM_X + _NB
_SEM_K = _SEM_X1 + _NS
_SEM_V = _SEM_K + _HKV
_SEM_MODA = _SEM_V + _HKV
_NSEM = _SEM_MODA + _NMA


def _kernel(x_hbm, k_hbm, v_hbm, wq_hbm, wo_hbm, wr_hbm, wg_hbm, wu_hbm, wd_hbm, c_hbm, wmod_hbm,
            out_hbm,
            x_v, h_a, h_b, k_v, v_v, wq_v, wo_v, wmod_v, wg_v, wu_v, wd_v, c_v, wr_v, wrf_v,
            o_a, o_b, a_a, a_b, out_v, h2_v, of_v, mod_v, modq_v, scol_v, best_v, bidx_v, fix_v, sems):
    h_buf, o_buf, a_buf = (h_a, h_b), (o_a, o_b), (a_a, a_b)

    def cp(src, dst, slot):
        return pltpu.make_async_copy(src, dst, sems.at[slot])

    d_c = cp(c_hbm, c_v, _SEM_C)

    def d_mod(i):
        return cp(wmod_hbm.at[:, pl.ds(i * _MC, _MC)], wmod_v.at[i],
                  _SEM_MODA + i if i < _NMA else _SEM_MODB)

    def d_k(g):
        return cp(k_hbm.at[g, pl.ds(_SK - _W, _W), :], k_v.at[g], _SEM_K + g)

    def d_v(g):
        return cp(v_hbm.at[g, pl.ds(_SK - _W, _W), :], v_v.at[g], _SEM_V + g)

    def d_x1(i):
        rows = pl.ds(pl.multiple_of(_M + i * _R, _R), _R)
        return cp(x_hbm.at[rows], x_v.at[rows], _SEM_X1 + i)

    def d_wq(j):
        return cp(wq_hbm.at[:, pl.ds(pl.multiple_of(j * _QC, _QC), _QC)], wq_v.at[j], _SEM_WQ + j)

    def d_x(b):
        return cp(x_hbm.at[pl.ds(b * _M, _M)], x_v.at[pl.ds(b * _M, _M)], _SEM_X + b)

    d_wr = cp(wr_hbm, wr_v, _SEM_WR)
    d_wg = cp(wg_hbm, wg_v, _SEM_WG)
    d_wu = cp(wu_hbm, wu_v, _SEM_WU)
    d_wd = cp(wd_hbm, wd_v, _SEM_WD)

    d_c.start()
    for i in range(_NMA):
        d_mod(i).start()
    d_x(0).start()
    for j in range(_NS):
        if j % _SPG == 0:
            d_k(j // _SPG).start()
            d_v(j // _SPG).start()
        d_wq(j).start()
        d_x1(j).start()
    for j in range(_NS):
        cp(wo_hbm.at[:, pl.ds(j * _NT, _NT)], wo_v.at[j], _SEM_WO).start()
    for b in range(2, _NB):
        d_x(b).start()
    d_wr.start()
    for i in range(_NMA, _NMC):
        d_mod(i).start()
    d_wg.start()
    d_wu.start()
    d_wd.start()

    def mod_chunk(i):
        cf = c_v[...].astype(_F32)
        sc = jnp.broadcast_to((cf * jax.nn.sigmoid(cf)).astype(_BF), (16, _D))
        m = jnp.dot(sc, wmod_v[i], preferred_element_type=_F32)
        mod_v[i] = m[0:8, :]

    def mod_chunk_vpu(i):
        col = scol_v[...]
        outs = []
        for t in range(_MC // 128):
            w = wmod_v[i, :, pl.ds(t * 128, 128)].astype(_F32)
            outs.append(jnp.sum(w * col, axis=0, keepdims=True))
        mod_v[i, 0:1, :] = jnp.concatenate(outs, axis=1)

    def modr(i):
        n = _D // _MC
        return jnp.concatenate([mod_v[n * i + u, 0:1, :] for u in range(n)], axis=1)

    def pack(xf):
        return pltpu.bitcast(xf.astype(_BF), jnp.uint32)

    def unpack(w):
        return pltpu.bitcast(w, _BF)

    def ln(xf):
        mu = jnp.mean(xf, axis=1, keepdims=True)
        d = xf - mu
        var = jnp.mean(d * d, axis=1, keepdims=True)
        return d * lax.rsqrt(var + _EPS)

    def ln1_slice(b, i):
        rows = pl.ds(pl.multiple_of(b * _M + i * _R, _R), _R)
        y = ln(x_v[rows, :].astype(_F32))
        h = y * modq_v[1:2, :] + modq_v[0:1, :]
        h_buf[b % 2][pl.ds(pl.multiple_of(i * (_R // 2), _R // 2), _R // 2), :] = pack(h)

    def tie(w, token):
        if token is None:
            return w
        return jnp.concatenate([w[0:8, 0:128] | token, w[0:8, 128:]], axis=1) if w.shape[0] == 8 else \
            jnp.concatenate([jnp.concatenate([w[0:8, 0:128] | token, w[0:8, 128:]], axis=1), w[8:]], axis=0)

    def qproj_head(b, j, hh, token=None):
        q = jnp.dot(unpack(tie(h_buf[b % 2][...], token)), wq_v[j, :, pl.ds(hh * _DH, _DH)],
                    preferred_element_type=_F32)
        return q.astype(_BF)

    def scores(j, q):
        return lax.dot_general(q, k_v[j // _SPG], (((1,), (1,)), ((), ())),
                               preferred_element_type=_F32)

    def softmax_pv(b, j, hh, s):
        m = jnp.max(s, axis=1, keepdims=True)
        p = jnp.exp2(s - m)
        l = jnp.sum(p, axis=1, keepdims=True)
        o = jnp.dot(p.astype(_BF), v_v[j // _SPG], preferred_element_type=_F32)
        r = pl.reciprocal(l, approx=True)
        r = r * (2.0 - l * r)
        o_buf[b % 2][j * (_HPS // _HPC) + hh // _HPC, :, pl.ds((hh % _HPC) * _DH, _DH)] = pack(o * r)

    def oproj_part(b, j, part, token=None):
        n = _NOC // _HPS
        lhs = jnp.concatenate([unpack(tie(o_buf[b % 2][part * n + jj], token if jj == 0 else None))
                               for jj in range(n)], axis=1)
        return jnp.dot(lhs, wo_v[j, pl.ds(part * n * _OW, n * _OW), :], preferred_element_type=_F32)

    def epilogue(b, i):
        lrows = pl.ds(pl.multiple_of(i * _R, _R), _R)
        row0 = pl.multiple_of(b * _M + i * _R, _R)
        rows = pl.ds(row0, _R)
        a = jnp.concatenate([a_buf[b % 2][jj, lrows, :] for jj in range(_NS)], axis=1)
        x1 = x_v[rows, :].astype(_F32) + modr(2) * a
        h2 = ln(x1) * (1.0 + modr(4)) + modr(3)
        o = x1 + modr(5) * h2
        out_v[rows, :] = o.astype(_BF)
        h2_v[rows, :] = h2
        of_v[rows, :] = o
        r = jnp.sum(h2 * wrf_v[...], axis=1, keepdims=True)
        r = jnp.broadcast_to(r, (_R, 128))
        ridx = row0 + lax.broadcasted_iota(jnp.int32, (_R, 128), 0)
        bv = best_v[...]
        bi = bidx_v[...]
        for s in range(_R // 8):
            rs = r[s * 8:(s + 1) * 8]
            upd = rs > bv
            bv = jnp.where(upd, rs, bv)
            bi = jnp.where(upd, ridx[s * 8:(s + 1) * 8], bi)
        best_v[...] = bv
        bidx_v[...] = bi
        return lax.shift_right_logical(bi, 31).astype(jnp.uint32)

    def block_phase(b):
        do_attn = True
        do_o = 1 <= b
        do_epi = 0 <= b - 2
        do_ln = b + 1 < _NB

        def step(j, carry):
            token = None
            if do_epi:
                token = epilogue(b - 2, j)
            if b == 0:
                @pl.when(j % _SPG == 0)
                def _():
                    d_k(j // _SPG).wait()
                    d_v(j // _SPG).wait()
                d_wq(j).wait()
                d_x1(j).wait()
            parts = []
            if do_attn:
                q = qproj_head(b, j, 0)
            for hh in range(_HPS):
                if do_o and hh == 0:
                    parts.append(oproj_part(b - 1, j, 0))
                if do_attn:
                    s = scores(j, q)
                    if hh + 1 < _HPS:
                        q = qproj_head(b, j, hh + 1, token if hh + 1 == _TIE_Q else None)
                    elif do_o:
                        parts.append(oproj_part(b - 1, j, 1, token if _TIE_Q is None else None))
                    softmax_pv(b, j, hh, s)
            if b == 1:
                for u in range((_NMC - _NMA) // _NS):
                    mod_chunk_vpu(_NMA + j * ((_NMC - _NMA) // _NS) + u)
            if do_ln:
                ln1_slice(b + 1, j)
            if do_o:
                for part in range(len(parts), _HPS):
                    parts.append(oproj_part(b - 1, j, part))
                a_buf[(b - 1) % 2][j] = functools.reduce(lambda u, w: u + w, parts)
            return carry
        lax.fori_loop(0, _NS, step, 0, unroll=1)

    def drain_phase(half):
        b = _NB - 1
        hm = _M // 2

        def step(jp, carry):
            if half == 0:
                tokens = [epilogue(b - 1, 2 * jp + u) for u in range(2)]
            else:
                tokens = [None, epilogue(b, jp)]
            rows_w = pl.ds(half * (hm // 2), hm // 2)
            n = _NOC // _HPS
            for u in range(2):
                j = 2 * jp + u
                parts = []
                for part in range(_HPS):
                    tk = tokens[u] if part == _TIE_D[half][u] else None
                    lhs = jnp.concatenate(
                        [unpack(tie(o_buf[b % 2][part * n + jj, rows_w, :], tk if jj == 0 else None))
                         for jj in range(n)], axis=1)
                    parts.append(jnp.dot(lhs, wo_v[j, pl.ds(part * n * _OW, n * _OW), :],
                                         preferred_element_type=_F32))
                a_buf[b % 2][j, pl.ds(half * hm, hm), :] = functools.reduce(lambda x_, y_: x_ + y_, parts)
            return carry
        lax.fori_loop(0, _NS // 2, step, 0)

    def out_copy(b):
        rows = pl.ds(b * _M, _M)
        return cp(out_v.at[rows], out_hbm.at[rows], _SEM_OUT)

    d_c.wait()
    cf = c_v[...].astype(_F32)
    sc = (cf * jax.nn.sigmoid(cf)).astype(_BF).astype(_F32)
    scol_v[...] = jnp.broadcast_to(sc, (128, _D)).T
    for i in range(_NMA):
        d_mod(i).wait()
        mod_chunk(i)
    modq_v[0:1, :] = modr(0) * _QSCALE
    modq_v[1:2, :] = (1.0 + modr(1)) * _QSCALE
    d_x(0).wait()
    for i in range(_NS):
        ln1_slice(0, i)
    best_v[...] = jnp.full((8, 128), -jnp.inf, _F32)
    bidx_v[...] = jnp.zeros((8, 128), jnp.int32)

    for b in range(_NB):
        if b == 1:
            pltpu.make_async_copy(wo_v, wo_v, sems.at[_SEM_WO]).wait()
            d_wr.wait()
            wrf_v[...] = wr_v[...].astype(_F32).reshape(1, _D)
            pltpu.make_async_copy(wmod_v.at[pl.ds(_NMA, _NMC - _NMA)],
                                  wmod_v.at[pl.ds(_NMA, _NMC - _NMA)], sems.at[_SEM_MODB]).wait()
        if 2 <= b + 1 < _NB:
            d_x(b + 1).wait()
        block_phase(b)
        if b >= 2:
            out_copy(b - 2).start()
    drain_phase(0)
    out_copy(_NB - 2).start()
    d_wg.wait()
    d_wu.wait()
    d_wd.wait()
    drain_phase(1)
    for i in range(_NS // 2, _NS):
        epilogue(_NB - 1, i)
    out_copy(_NB - 1).start()

    bv = best_v[...]
    bi = bidx_v[...]
    rmax = jnp.max(bv, axis=0, keepdims=True)
    cand = jnp.where(bv == rmax, bi, _S)
    sel = jnp.min(cand)
    sel = jnp.clip(sel, 0, _S - 1)
    gate_r = jax.nn.sigmoid(rmax[:, 0:1])

    xs = h2_v[pl.ds(sel, 1), :].astype(_BF)
    xs = jnp.broadcast_to(xs, (16, _D))
    g = jnp.dot(xs, wg_v[...], preferred_element_type=_F32)
    u = jnp.dot(xs, wu_v[...], preferred_element_type=_F32)
    act = (g * jax.nn.sigmoid(g) * u).astype(_BF)
    y = functools.reduce(lambda u_, w_: u_ + w_, [
        jnp.dot(act[:, i * 512:(i + 1) * 512], wd_v[pl.ds(i * 512, 512), :],
                preferred_element_type=_F32) for i in range(_F // 512)])[0:1, :]
    row = of_v[pl.ds(sel, 1), :] + modr(5) * (y * gate_r)

    base = pl.multiple_of((sel // 16) * 16, 16)
    tile = of_v[pl.ds(base, 16), :]
    rid = base + lax.broadcasted_iota(jnp.int32, (16, _D), 0)
    fix_v[...] = jnp.where(rid == sel, row, tile).astype(_BF)

    pltpu.make_async_copy(out_v, out_hbm, sems.at[_SEM_OUT]).wait()
    d_fix = cp(fix_v, out_hbm.at[pl.ds(base, 16)], _SEM_FIX)
    d_fix.start()
    d_fix.wait()


@jax.jit
def pallas_adaLN_cond__sliding_block_cached__moe_arch_mod__prompt_kernel(
    A_x: jax.Array,
    A_k_cache: jax.Array,
    A_v_cache: jax.Array,
    A_wq: jax.Array,
    A_wo: jax.Array,
    B_x: jax.Array,
    B_w_r: jax.Array,
    B_w_gate: jax.Array,
    B_w_up: jax.Array,
    B_w_down: jax.Array,
    c: jax.Array,
    w_mod: jax.Array,
):
    del B_x
    x = A_x.reshape(_S, _D)
    k = A_k_cache.reshape(_HKV, _SK, _DH)
    v = A_v_cache.reshape(_HKV, _SK, _DH)

    any_spec = pl.BlockSpec(memory_space=pl.ANY)
    out = pl.pallas_call(
        _kernel,
        out_shape=jax.ShapeDtypeStruct((_S, _D), _BF),
        in_specs=[any_spec] * 11,
        out_specs=any_spec,
        scratch_shapes=[
            pltpu.VMEM((_S, _D), _BF),
            pltpu.VMEM((_M // 2, _D), jnp.uint32),
            pltpu.VMEM((_M // 2, _D), jnp.uint32),
            pltpu.VMEM((_HKV, _W, _DH), _BF),
            pltpu.VMEM((_HKV, _W, _DH), _BF),
            pltpu.VMEM((_NS, _D, _QC), _BF),
            pltpu.VMEM((_NS, _HQ * _DH, _NT), _BF),
            pltpu.VMEM((_NMC, _D, _MC), _BF),
            pltpu.VMEM((_D, _F), _BF),
            pltpu.VMEM((_D, _F), _BF),
            pltpu.VMEM((_F, _D), _BF),
            pltpu.VMEM((1, _D), _BF),
            pltpu.VMEM((_D,), _BF),
            pltpu.VMEM((1, _D), _F32),
            pltpu.VMEM((_NOC, _M // 2, _OW), jnp.uint32),
            pltpu.VMEM((_NOC, _M // 2, _OW), jnp.uint32),
            pltpu.VMEM((_NS, _M, _NT), _F32),
            pltpu.VMEM((_NS, _M, _NT), _F32),
            pltpu.VMEM((_S, _D), _BF),
            pltpu.VMEM((_S, _D), _F32),
            pltpu.VMEM((_S, _D), _F32),
            pltpu.VMEM((_NMC, 8, _MC), _F32),
            pltpu.VMEM((2, _D), _F32),
            pltpu.VMEM((_D, 128), _F32),
            pltpu.VMEM((8, 128), _F32),
            pltpu.VMEM((8, 128), jnp.int32),
            pltpu.VMEM((16, _D), _BF),
            pltpu.SemaphoreType.DMA((_NSEM,)),
        ],
        compiler_params=pltpu.CompilerParams(vmem_limit_bytes=110 * 1024 * 1024),
    )(x, k, v, A_wq, A_wo, B_w_r, B_w_gate, B_w_up, B_w_down, c, w_mod)
    return out.reshape(1, _S, _D)
```

```python
import functools

import jax
import jax.numpy as jnp
from jax import lax
from jax.experimental import pallas as pl
from jax.experimental.pallas import tpu as pltpu

_S = 2048
_D = 1024
_HQ = 32
_HKV = 4
_DH = 128
_SK = 2048
_W = min(4096, max(256, _SK // 4))
_F = 3584
_EPS = 1e-5

_M = 512
_NB = _S // _M
_HPS = 4
_NS = _HQ // _HPS
_R = _M // _NS
_QC = _HPS * _DH
_NT = _D // _NS
_SPG = _NS // _HKV
_OW = 512
_NOC = _HQ * _DH // _OW
_HPC = _OW // _DH
_TIE_Q = 1
_UNIFORM = False
_TIE_D = ((2, 1), (None, 2))
_MC = 512
_NMC = 6 * _D // _MC
_NMA = 2 * _D // _MC
assert (_NMC - _NMA) % _NS == 0

_LOG2E = 1.4426950408889634
_QSCALE = (_DH ** -0.5) * _LOG2E

_BF = jnp.bfloat16
_F32 = jnp.float32

_SEM_C, _SEM_WR, _SEM_MODB, _SEM_WO, _SEM_WG, _SEM_WU, _SEM_WD = 0, 1, 2, 3, 4, 5, 6
_SEM_OUT, _SEM_FIX = 7, 8
_SEM_WQ = 9
_SEM_X = _SEM_WQ + _NS
_SEM_X1 = _SEM_X + _NB
_SEM_K = _SEM_X1 + _NS
_SEM_V = _SEM_K + _HKV
_SEM_MODA = _SEM_V + _HKV
_NSEM = _SEM_MODA + _NMA


def _kernel(x_hbm, k_hbm, v_hbm, wq_hbm, wo_hbm, wr_hbm, wg_hbm, wu_hbm, wd_hbm, c_hbm, wmod_hbm,
            out_hbm,
            x_v, h_a, h_b, k_v, v_v, wq_v, wo_v, wmod_v, wg_v, wu_v, wd_v, c_v, wr_v, wrf_v,
            o_a, o_b, a_a, a_b, out_v, brow_v, mod_v, modq_v, scol_v, best_v, bidx_v, fix_v, sems):
    h_buf, o_buf, a_buf = (h_a, h_b), (o_a, o_b), (a_a, a_b)

    def cp(src, dst, slot):
        return pltpu.make_async_copy(src, dst, sems.at[slot])

    d_c = cp(c_hbm, c_v, _SEM_C)

    def d_mod(i):
        return cp(wmod_hbm.at[:, pl.ds(i * _MC, _MC)], wmod_v.at[i],
                  _SEM_MODA + i if i < _NMA else _SEM_MODB)

    def d_k(g):
        return cp(k_hbm.at[g, pl.ds(_SK - _W, _W), :], k_v.at[g], _SEM_K + g)

    def d_v(g):
        return cp(v_hbm.at[g, pl.ds(_SK - _W, _W), :], v_v.at[g], _SEM_V + g)

    def d_x1(i):
        rows = pl.ds(pl.multiple_of(_M + i * _R, _R), _R)
        return cp(x_hbm.at[rows], x_v.at[rows], _SEM_X1 + i)

    def d_wq(j):
        return cp(wq_hbm.at[:, pl.ds(pl.multiple_of(j * _QC, _QC), _QC)], wq_v.at[j], _SEM_WQ + j)

    def d_x(b):
        return cp(x_hbm.at[pl.ds(b * _M, _M)], x_v.at[pl.ds(b * _M, _M)], _SEM_X + b)

    d_wr = cp(wr_hbm, wr_v, _SEM_WR)
    d_wg = cp(wg_hbm, wg_v, _SEM_WG)
    d_wu = cp(wu_hbm, wu_v, _SEM_WU)
    d_wd = cp(wd_hbm, wd_v, _SEM_WD)

    d_c.start()
    for i in range(_NMA):
        d_mod(i).start()
    d_x(0).start()
    for j in range(_NS):
        if j % _SPG == 0:
            d_k(j // _SPG).start()
            d_v(j // _SPG).start()
        d_wq(j).start()
        d_x1(j).start()
    for j in range(_NS):
        cp(wo_hbm.at[:, pl.ds(j * _NT, _NT)], wo_v.at[j], _SEM_WO).start()
    for b in range(2, _NB):
        d_x(b).start()
    d_wr.start()
    for i in range(_NMA, _NMC):
        d_mod(i).start()
    d_wg.start()
    d_wu.start()
    d_wd.start()

    def mod_chunk(i):
        cf = c_v[...].astype(_F32)
        sc = jnp.broadcast_to((cf * jax.nn.sigmoid(cf)).astype(_BF), (16, _D))
        m = jnp.dot(sc, wmod_v[i], preferred_element_type=_F32)
        mod_v[i] = m[0:8, :]

    def mod_chunk_vpu(i):
        col = scol_v[...]
        outs = []
        for t in range(_MC // 128):
            w = wmod_v[i, :, pl.ds(t * 128, 128)].astype(_F32)
            outs.append(jnp.sum(w * col, axis=0, keepdims=True))
        mod_v[i, 0:1, :] = jnp.concatenate(outs, axis=1)

    def modr(i):
        n = _D // _MC
        return jnp.concatenate([mod_v[n * i + u, 0:1, :] for u in range(n)], axis=1)

    def pack(xf):
        return pltpu.bitcast(xf.astype(_BF), jnp.uint32)

    def unpack(w):
        return pltpu.bitcast(w, _BF)

    def ln(xf):
        mu = jnp.mean(xf, axis=1, keepdims=True)
        d = xf - mu
        var = jnp.mean(d * d, axis=1, keepdims=True)
        return d * lax.rsqrt(var + _EPS)

    def ln1_slice(b, i):
        rows = pl.ds(pl.multiple_of(b * _M + i * _R, _R), _R)
        y = ln(x_v[rows, :].astype(_F32))
        h = y * modq_v[1:2, :] + modq_v[0:1, :]
        h_buf[b % 2][pl.ds(pl.multiple_of(i * (_R // 2), _R // 2), _R // 2), :] = pack(h)

    def tie(w, token):
        if token is None:
            return w
        return jnp.concatenate([w[0:8, 0:128] | token, w[0:8, 128:]], axis=1) if w.shape[0] == 8 else \
            jnp.concatenate([jnp.concatenate([w[0:8, 0:128] | token, w[0:8, 128:]], axis=1), w[8:]], axis=0)

    def qproj_head(b, j, hh, token=None):
        q = jnp.dot(unpack(tie(h_buf[b % 2][...], token)), wq_v[j, :, pl.ds(hh * _DH, _DH)],
                    preferred_element_type=_F32)
        return q.astype(_BF)

    def scores(j, q):
        return lax.dot_general(q, k_v[j // _SPG], (((1,), (1,)), ((), ())),
                               preferred_element_type=_F32)

    def softmax_pv(b, j, hh, s):
        m = jnp.max(s, axis=1, keepdims=True)
        p = jnp.exp2(s - m)
        l = jnp.sum(p, axis=1, keepdims=True)
        o = jnp.dot(p.astype(_BF), v_v[j // _SPG], preferred_element_type=_F32)
        r = pl.reciprocal(l, approx=True)
        r = r * (2.0 - l * r)
        o_buf[b % 2][j * (_HPS // _HPC) + hh // _HPC, :, pl.ds((hh % _HPC) * _DH, _DH)] = pack(o * r)

    def oproj_part(b, j, part, token=None):
        n = _NOC // _HPS
        lhs = jnp.concatenate([unpack(tie(o_buf[b % 2][part * n + jj], token if jj == 0 else None))
                               for jj in range(n)], axis=1)
        return jnp.dot(lhs, wo_v[j, pl.ds(part * n * _OW, n * _OW), :], preferred_element_type=_F32)

    def epilogue(b, i):
        lrows = pl.ds(pl.multiple_of(i * _R, _R), _R)
        row0 = pl.multiple_of(b * _M + i * _R, _R)
        rows = pl.ds(row0, _R)
        a = jnp.concatenate([a_buf[b % 2][jj, lrows, :] for jj in range(_NS)], axis=1)
        x1 = x_v[rows, :].astype(_F32) + modr(2) * a
        h2 = ln(x1) * (1.0 + modr(4)) + modr(3)
        o = x1 + modr(5) * h2
        out_v[rows, :] = o.astype(_BF)
        r = jnp.sum(h2 * wrf_v[...], axis=1, keepdims=True)
        r = jnp.broadcast_to(r, (_R, 128))
        ridx = row0 + lax.broadcasted_iota(jnp.int32, (_R, 128), 0)
        bv = best_v[...]
        bi = bidx_v[...]
        bh = brow_v[0]
        bo = brow_v[1]
        for s in range(_R // 8):
            grp = slice(s * 8, (s + 1) * 8)
            upd = r[grp] > bv
            bv = jnp.where(upd, r[grp], bv)
            bi = jnp.where(upd, ridx[grp], bi)
            upd_w = jnp.concatenate([upd] * (_D // 128), axis=1)
            bh = jnp.where(upd_w, h2[grp], bh)
            bo = jnp.where(upd_w, o[grp], bo)
        best_v[...] = bv
        bidx_v[...] = bi
        brow_v[0] = bh
        brow_v[1] = bo
        return lax.shift_right_logical(bi, 31).astype(jnp.uint32)

    def block_phase(b):
        do_attn = True
        do_o = 1 <= b
        do_epi = 0 <= b - 2
        do_ln = b + 1 < _NB

        def step(j, carry):
            token = None
            if do_epi:
                token = epilogue(b - 2, j)
            if b == 0:
                @pl.when(j % _SPG == 0)
                def _():
                    d_k(j // _SPG).wait()
                    d_v(j // _SPG).wait()
                d_wq(j).wait()
                d_x1(j).wait()
            parts = []
            q = qproj_head(b, j, 0)
            if do_o:
                parts.append(oproj_part(b - 1, j, 0))
            for hh in range(_HPS):
                s = scores(j, q)
                if hh + 1 < _HPS:
                    q = qproj_head(b, j, hh + 1, token if hh + 1 == _TIE_Q else None)
                elif do_o:
                    parts.append(oproj_part(b - 1, j, len(parts)))
                softmax_pv(b, j, hh, s)
                if do_o and _UNIFORM and hh < _HPS - 2:
                    parts.append(oproj_part(b - 1, j, len(parts)))
            if b == 1:
                for u in range((_NMC - _NMA) // _NS):
                    mod_chunk_vpu(_NMA + j * ((_NMC - _NMA) // _NS) + u)
            if do_ln:
                ln1_slice(b + 1, j)
            if do_o:
                for part in range(len(parts), _HPS):
                    parts.append(oproj_part(b - 1, j, part))
                a_buf[(b - 1) % 2][j] = functools.reduce(lambda u, w: u + w, parts)
            return carry
        lax.fori_loop(0, _NS, step, 0, unroll=1)

    def drain_phase(half):
        b = _NB - 1
        hm = _M // 2

        def step(jp, carry):
            if half == 0:
                tokens = [epilogue(b - 1, 2 * jp + u) for u in range(2)]
            else:
                tokens = [None, epilogue(b, jp)]
            rows_w = pl.ds(half * (hm // 2), hm // 2)
            n = _NOC // _HPS
            for u in range(2):
                j = 2 * jp + u
                parts = []
                for part in range(_HPS):
                    tk = tokens[u] if part == _TIE_D[half][u] else None
                    lhs = jnp.concatenate(
                        [unpack(tie(o_buf[b % 2][part * n + jj, rows_w, :], tk if jj == 0 else None))
                         for jj in range(n)], axis=1)
                    parts.append(jnp.dot(lhs, wo_v[j, pl.ds(part * n * _OW, n * _OW), :],
                                         preferred_element_type=_F32))
                a_buf[b % 2][j, pl.ds(half * hm, hm), :] = functools.reduce(lambda x_, y_: x_ + y_, parts)
            return carry
        lax.fori_loop(0, _NS // 2, step, 0)

    def out_copy(b):
        rows = pl.ds(b * _M, _M)
        return cp(out_v.at[rows], out_hbm.at[rows], _SEM_OUT)

    d_c.wait()
    cf = c_v[...].astype(_F32)
    sc = (cf * jax.nn.sigmoid(cf)).astype(_BF).astype(_F32)
    scol_v[...] = jnp.broadcast_to(sc, (128, _D)).T
    for i in range(_NMA):
        d_mod(i).wait()
        mod_chunk(i)
    modq_v[0:1, :] = modr(0) * _QSCALE
    modq_v[1:2, :] = (1.0 + modr(1)) * _QSCALE
    d_x(0).wait()
    for i in range(_NS):
        ln1_slice(0, i)
    best_v[...] = jnp.full((8, 128), -jnp.inf, _F32)
    bidx_v[...] = jnp.zeros((8, 128), jnp.int32)
    brow_v[...] = jnp.zeros((2, 8, _D), _F32)

    for b in range(_NB):
        if b == 1:
            pltpu.make_async_copy(wo_v, wo_v, sems.at[_SEM_WO]).wait()
            d_wr.wait()
            wrf_v[...] = wr_v[...].astype(_F32).reshape(1, _D)
            pltpu.make_async_copy(wmod_v.at[pl.ds(_NMA, _NMC - _NMA)],
                                  wmod_v.at[pl.ds(_NMA, _NMC - _NMA)], sems.at[_SEM_MODB]).wait()
        if 2 <= b + 1 < _NB:
            d_x(b + 1).wait()
        block_phase(b)
        if b >= 2:
            out_copy(b - 2).start()
    drain_phase(0)
    out_copy(_NB - 2).start()
    d_wg.wait()
    d_wu.wait()
    d_wd.wait()
    drain_phase(1)
    for i in range(_NS // 2, _NS):
        epilogue(_NB - 1, i)
    out_copy(_NB - 1).start()

    bv = best_v[...]
    bi = bidx_v[...]
    rmax = jnp.max(bv, axis=0, keepdims=True)
    cand = jnp.where(bv == rmax, bi, _S)
    sel = jnp.min(cand)
    sel = jnp.clip(sel, 0, _S - 1)
    gate_r = jax.nn.sigmoid(rmax[:, 0:1])

    cls = pl.ds(sel % 8, 1)
    xs = jnp.broadcast_to(brow_v[0, cls, :].astype(_BF), (16, _D))
    g = jnp.dot(xs, wg_v[...], preferred_element_type=_F32)
    u = jnp.dot(xs, wu_v[...], preferred_element_type=_F32)
    act = (g * jax.nn.sigmoid(g) * u).astype(_BF)
    y = functools.reduce(lambda u_, w_: u_ + w_, [
        jnp.dot(act[:, i * 512:(i + 1) * 512], wd_v[pl.ds(i * 512, 512), :],
                preferred_element_type=_F32) for i in range(_F // 512)])[0:1, :]
    row = brow_v[1, cls, :] + modr(5) * (y * gate_r)

    base = pl.multiple_of((sel // 16) * 16, 16)
    rid = base + lax.broadcasted_iota(jnp.int32, (16, _D), 0)
    fix_v[...] = jnp.where(rid == sel, row, out_v[pl.ds(base, 16), :].astype(_F32)).astype(_BF)

    pltpu.make_async_copy(out_v, out_hbm, sems.at[_SEM_OUT]).wait()
    d_fix = cp(fix_v, out_hbm.at[pl.ds(base, 16)], _SEM_FIX)
    d_fix.start()
    d_fix.wait()


@jax.jit
def pallas_adaLN_cond__sliding_block_cached__moe_arch_mod__prompt_kernel(
    A_x: jax.Array,
    A_k_cache: jax.Array,
    A_v_cache: jax.Array,
    A_wq: jax.Array,
    A_wo: jax.Array,
    B_x: jax.Array,
    B_w_r: jax.Array,
    B_w_gate: jax.Array,
    B_w_up: jax.Array,
    B_w_down: jax.Array,
    c: jax.Array,
    w_mod: jax.Array,
):
    del B_x
    x = A_x.reshape(_S, _D)
    k = A_k_cache.reshape(_HKV, _SK, _DH)
    v = A_v_cache.reshape(_HKV, _SK, _DH)

    any_spec = pl.BlockSpec(memory_space=pl.ANY)
    out = pl.pallas_call(
        _kernel,
        out_shape=jax.ShapeDtypeStruct((_S, _D), _BF),
        in_specs=[any_spec] * 11,
        out_specs=any_spec,
        scratch_shapes=[
            pltpu.VMEM((_S, _D), _BF),
            pltpu.VMEM((_M // 2, _D), jnp.uint32),
            pltpu.VMEM((_M // 2, _D), jnp.uint32),
            pltpu.VMEM((_HKV, _W, _DH), _BF),
            pltpu.VMEM((_HKV, _W, _DH), _BF),
            pltpu.VMEM((_NS, _D, _QC), _BF),
            pltpu.VMEM((_NS, _HQ * _DH, _NT), _BF),
            pltpu.VMEM((_NMC, _D, _MC), _BF),
            pltpu.VMEM((_D, _F), _BF),
            pltpu.VMEM((_D, _F), _BF),
            pltpu.VMEM((_F, _D), _BF),
            pltpu.VMEM((1, _D), _BF),
            pltpu.VMEM((_D,), _BF),
            pltpu.VMEM((1, _D), _F32),
            pltpu.VMEM((_NOC, _M // 2, _OW), jnp.uint32),
            pltpu.VMEM((_NOC, _M // 2, _OW), jnp.uint32),
            pltpu.VMEM((_NS, _M, _NT), _F32),
            pltpu.VMEM((_NS, _M, _NT), _F32),
            pltpu.VMEM((_S, _D), _BF),
            pltpu.VMEM((2, 8, _D), _F32),
            pltpu.VMEM((_NMC, 8, _MC), _F32),
            pltpu.VMEM((2, _D), _F32),
            pltpu.VMEM((_D, 128), _F32),
            pltpu.VMEM((8, 128), _F32),
            pltpu.VMEM((8, 128), jnp.int32),
            pltpu.VMEM((16, _D), _BF),
            pltpu.SemaphoreType.DMA((_NSEM,)),
        ],
        compiler_params=pltpu.CompilerParams(vmem_limit_bytes=110 * 1024 * 1024),
    )(x, k, v, A_wq, A_wo, B_w_r, B_w_gate, B_w_up, B_w_down, c, w_mod)
    return out.reshape(1, _S, _D)
```

```python
import functools

import jax
import jax.numpy as jnp
from jax import lax
from jax.experimental import pallas as pl
from jax.experimental.pallas import tpu as pltpu

_S = 2048
_D = 1024
_HQ = 32
_HKV = 4
_DH = 128
_SK = 2048
_W = min(4096, max(256, _SK // 4))
_F = 3584
_EPS = 1e-5

_M = 512
_NB = _S // _M
_HPS = 4
_NS = _HQ // _HPS
_R = _M // _NS
_QC = _HPS * _DH
_NT = _D // _NS
_SPG = _NS // _HKV
_OW = 512
_NOC = _HQ * _DH // _OW
_HPC = _OW // _DH
_TIE_Q = 1
_UNIFORM = False
_TIE_D = ((2, 1), (None, 2))
_FC = 256
_MC = 512
_NMC = 6 * _D // _MC
_NMA = 2 * _D // _MC
assert (_NMC - _NMA) % _NS == 0

_LOG2E = 1.4426950408889634
_QSCALE = (_DH ** -0.5) * _LOG2E

_BF = jnp.bfloat16
_F32 = jnp.float32

_SEM_C, _SEM_WR, _SEM_MODB, _SEM_WO, _SEM_WG, _SEM_WU, _SEM_WD = 0, 1, 2, 3, 4, 5, 6
_SEM_OUT, _SEM_FIX = 7, 8
_SEM_WQ = 9
_SEM_X = _SEM_WQ + _NS
_SEM_X1 = _SEM_X + _NB
_SEM_K = _SEM_X1 + _NS
_SEM_V = _SEM_K + _HKV
_SEM_MODA = _SEM_V + _HKV
_NSEM = _SEM_MODA + _NMA


def _kernel(x_hbm, k_hbm, v_hbm, wq_hbm, wo_hbm, wr_hbm, wg_hbm, wu_hbm, wd_hbm, c_hbm, wmod_hbm,
            out_hbm,
            x_v, h_a, h_b, k_v, v_v, wq_v, wo_v, wmod_v, wg_v, wu_v, wd_v, c_v, wr_v, wrf_v,
            o_a, o_b, a_a, a_b, out_v, brow_v, mod_v, modq_v, scol_v, best_v, bidx_v, fix_v, sems):
    h_buf, o_buf, a_buf = (h_a, h_b), (o_a, o_b), (a_a, a_b)

    def cp(src, dst, slot):
        return pltpu.make_async_copy(src, dst, sems.at[slot])

    d_c = cp(c_hbm, c_v, _SEM_C)

    def d_mod(i):
        return cp(wmod_hbm.at[:, pl.ds(i * _MC, _MC)], wmod_v.at[i],
                  _SEM_MODA + i if i < _NMA else _SEM_MODB)

    def d_k(g):
        return cp(k_hbm.at[g, pl.ds(_SK - _W, _W), :], k_v.at[g], _SEM_K + g)

    def d_v(g):
        return cp(v_hbm.at[g, pl.ds(_SK - _W, _W), :], v_v.at[g], _SEM_V + g)

    def d_x1(i):
        rows = pl.ds(pl.multiple_of(_M + i * _R, _R), _R)
        return cp(x_hbm.at[rows], x_v.at[rows], _SEM_X1 + i)

    def d_wq(j):
        return cp(wq_hbm.at[:, pl.ds(pl.multiple_of(j * _QC, _QC), _QC)], wq_v.at[j], _SEM_WQ + j)

    def d_x(b):
        return cp(x_hbm.at[pl.ds(b * _M, _M)], x_v.at[pl.ds(b * _M, _M)], _SEM_X + b)

    d_wr = cp(wr_hbm, wr_v, _SEM_WR)
    d_wg = cp(wg_hbm, wg_v, _SEM_WG)
    d_wu = cp(wu_hbm, wu_v, _SEM_WU)
    d_wd = cp(wd_hbm, wd_v, _SEM_WD)

    d_c.start()
    for i in range(_NMA):
        d_mod(i).start()
    d_x(0).start()
    for j in range(_NS):
        if j % _SPG == 0:
            d_k(j // _SPG).start()
            d_v(j // _SPG).start()
        d_wq(j).start()
        d_x1(j).start()
    for j in range(_NS):
        cp(wo_hbm.at[:, pl.ds(j * _NT, _NT)], wo_v.at[j], _SEM_WO).start()
    for b in range(2, _NB):
        d_x(b).start()
    d_wr.start()
    for i in range(_NMA, _NMC):
        d_mod(i).start()
    d_wg.start()
    d_wu.start()
    d_wd.start()

    def mod_chunk(i):
        cf = c_v[...].astype(_F32)
        sc = jnp.broadcast_to((cf * jax.nn.sigmoid(cf)).astype(_BF), (16, _D))
        m = jnp.dot(sc, wmod_v[i], preferred_element_type=_F32)
        mod_v[i] = m[0:8, :]

    def mod_chunk_vpu(i):
        col = scol_v[...]
        outs = []
        for t in range(_MC // 128):
            w = wmod_v[i, :, pl.ds(t * 128, 128)].astype(_F32)
            outs.append(jnp.sum(w * col, axis=0, keepdims=True))
        mod_v[i, 0:1, :] = jnp.concatenate(outs, axis=1)

    def modr(i):
        n = _D // _MC
        return jnp.concatenate([mod_v[n * i + u, 0:1, :] for u in range(n)], axis=1)

    def pack(xf):
        return pltpu.bitcast(xf.astype(_BF), jnp.uint32)

    def unpack(w):
        return pltpu.bitcast(w, _BF)

    def ln(xf):
        mu = jnp.mean(xf, axis=1, keepdims=True)
        d = xf - mu
        var = jnp.mean(d * d, axis=1, keepdims=True)
        return d * lax.rsqrt(var + _EPS)

    def ln1_slice(b, i):
        rows = pl.ds(pl.multiple_of(b * _M + i * _R, _R), _R)
        y = ln(x_v[rows, :].astype(_F32))
        h = y * modq_v[1:2, :] + modq_v[0:1, :]
        h_buf[b % 2][pl.ds(pl.multiple_of(i * (_R // 2), _R // 2), _R // 2), :] = pack(h)

    def tie(w, token):
        if token is None:
            return w
        return jnp.concatenate([w[0:8, 0:128] | token, w[0:8, 128:]], axis=1) if w.shape[0] == 8 else \
            jnp.concatenate([jnp.concatenate([w[0:8, 0:128] | token, w[0:8, 128:]], axis=1), w[8:]], axis=0)

    def qproj_head(b, j, hh, token=None):
        q = jnp.dot(unpack(tie(h_buf[b % 2][...], token)), wq_v[j, :, pl.ds(hh * _DH, _DH)],
                    preferred_element_type=_F32)
        return q.astype(_BF)

    def scores(j, q):
        return lax.dot_general(q, k_v[j // _SPG], (((1,), (1,)), ((), ())),
                               preferred_element_type=_F32)

    def softmax_pv(b, j, hh, s):
        m = jnp.max(s, axis=1, keepdims=True)
        p = jnp.exp2(s - m)
        l = jnp.sum(p, axis=1, keepdims=True)
        o = jnp.dot(p.astype(_BF), v_v[j // _SPG], preferred_element_type=_F32)
        r = pl.reciprocal(l, approx=True)
        r = r * (2.0 - l * r)
        o_buf[b % 2][j * (_HPS // _HPC) + hh // _HPC, :, pl.ds((hh % _HPC) * _DH, _DH)] = pack(o * r)

    def oproj_part(b, j, part, token=None):
        n = _NOC // _HPS
        lhs = jnp.concatenate([unpack(tie(o_buf[b % 2][part * n + jj], token if jj == 0 else None))
                               for jj in range(n)], axis=1)
        return jnp.dot(lhs, wo_v[j, pl.ds(part * n * _OW, n * _OW), :], preferred_element_type=_F32)

    def epilogue(b, i):
        lrows = pl.ds(pl.multiple_of(i * _R, _R), _R)
        row0 = pl.multiple_of(b * _M + i * _R, _R)
        rows = pl.ds(row0, _R)
        a = jnp.concatenate([a_buf[b % 2][jj, lrows, :] for jj in range(_NS)], axis=1)
        x1 = x_v[rows, :].astype(_F32) + modr(2) * a
        h2 = ln(x1) * (1.0 + modr(4)) + modr(3)
        o = x1 + modr(5) * h2
        out_v[rows, :] = o.astype(_BF)
        r = jnp.sum(h2 * wrf_v[...], axis=1, keepdims=True)
        r = jnp.broadcast_to(r, (_R, 128))
        ridx = row0 + lax.broadcasted_iota(jnp.int32, (_R, 128), 0)
        bv = best_v[...]
        bi = bidx_v[...]
        bh = brow_v[0]
        bo = brow_v[1]
        for s in range(_R // 8):
            grp = slice(s * 8, (s + 1) * 8)
            upd = r[grp] > bv
            bv = jnp.where(upd, r[grp], bv)
            bi = jnp.where(upd, ridx[grp], bi)
            upd_w = jnp.concatenate([upd] * (_D // 128), axis=1)
            bh = jnp.where(upd_w, h2[grp], bh)
            bo = jnp.where(upd_w, o[grp], bo)
        best_v[...] = bv
        bidx_v[...] = bi
        brow_v[0] = bh
        brow_v[1] = bo
        return lax.shift_right_logical(bi, 31).astype(jnp.uint32)

    def block_phase(b):
        do_attn = True
        do_o = 1 <= b
        do_epi = 0 <= b - 2
        do_ln = b + 1 < _NB

        def step(j, carry):
            token = None
            if do_epi:
                token = epilogue(b - 2, j)
            if b == 0:
                @pl.when(j % _SPG == 0)
                def _():
                    d_k(j // _SPG).wait()
                    d_v(j // _SPG).wait()
                d_wq(j).wait()
                d_x1(j).wait()
            parts = []
            q = qproj_head(b, j, 0)
            if do_o:
                parts.append(oproj_part(b - 1, j, 0))
            for hh in range(_HPS):
                s = scores(j, q)
                if hh + 1 < _HPS:
                    q = qproj_head(b, j, hh + 1, token if hh + 1 == _TIE_Q else None)
                elif do_o:
                    parts.append(oproj_part(b - 1, j, len(parts)))
                softmax_pv(b, j, hh, s)
                if do_o and _UNIFORM and hh < _HPS - 2:
                    parts.append(oproj_part(b - 1, j, len(parts)))
            if b == 1:
                for u in range((_NMC - _NMA) // _NS):
                    mod_chunk_vpu(_NMA + j * ((_NMC - _NMA) // _NS) + u)
            if do_ln:
                ln1_slice(b + 1, j)
            if do_o:
                for part in range(len(parts), _HPS):
                    parts.append(oproj_part(b - 1, j, part))
                a_buf[(b - 1) % 2][j] = functools.reduce(lambda u, w: u + w, parts)
            return carry
        lax.fori_loop(0, _NS, step, 0, unroll=1)

    def drain_phase(half):
        b = _NB - 1
        hm = _M // 2

        def step(jp, carry):
            if half == 0:
                tokens = [epilogue(b - 1, 2 * jp + u) for u in range(2)]
            else:
                tokens = [None, epilogue(b, jp)]
            rows_w = pl.ds(half * (hm // 2), hm // 2)
            n = _NOC // _HPS
            for u in range(2):
                j = 2 * jp + u
                parts = []
                for part in range(_HPS):
                    tk = tokens[u] if part == _TIE_D[half][u] else None
                    lhs = jnp.concatenate(
                        [unpack(tie(o_buf[b % 2][part * n + jj, rows_w, :], tk if jj == 0 else None))
                         for jj in range(n)], axis=1)
                    parts.append(jnp.dot(lhs, wo_v[j, pl.ds(part * n * _OW, n * _OW), :],
                                         preferred_element_type=_F32))
                a_buf[b % 2][j, pl.ds(half * hm, hm), :] = functools.reduce(lambda x_, y_: x_ + y_, parts)
            return carry
        lax.fori_loop(0, _NS // 2, step, 0)

    def out_copy(b):
        rows = pl.ds(b * _M, _M)
        return cp(out_v.at[rows], out_hbm.at[rows], _SEM_OUT)

    d_c.wait()
    cf = c_v[...].astype(_F32)
    sc = (cf * jax.nn.sigmoid(cf)).astype(_BF).astype(_F32)
    scol_v[...] = jnp.broadcast_to(sc, (128, _D)).T
    for i in range(_NMA):
        d_mod(i).wait()
        mod_chunk(i)
    modq_v[0:1, :] = modr(0) * _QSCALE
    modq_v[1:2, :] = (1.0 + modr(1)) * _QSCALE
    d_x(0).wait()
    for i in range(_NS):
        ln1_slice(0, i)
    best_v[...] = jnp.full((8, 128), -jnp.inf, _F32)
    bidx_v[...] = jnp.zeros((8, 128), jnp.int32)
    brow_v[...] = jnp.zeros((2, 8, _D), _F32)

    for b in range(_NB):
        if b == 1:
            pltpu.make_async_copy(wo_v, wo_v, sems.at[_SEM_WO]).wait()
            d_wr.wait()
            wrf_v[...] = wr_v[...].astype(_F32).reshape(1, _D)
            pltpu.make_async_copy(wmod_v.at[pl.ds(_NMA, _NMC - _NMA)],
                                  wmod_v.at[pl.ds(_NMA, _NMC - _NMA)], sems.at[_SEM_MODB]).wait()
        if 2 <= b + 1 < _NB:
            d_x(b + 1).wait()
        block_phase(b)
        if b >= 2:
            out_copy(b - 2).start()
    drain_phase(0)
    out_copy(_NB - 2).start()
    d_wg.wait()
    d_wu.wait()
    d_wd.wait()
    drain_phase(1)
    for i in range(_NS // 2, _NS):
        epilogue(_NB - 1, i)
    out_copy(_NB - 1).start()

    bv = best_v[...]
    bi = bidx_v[...]
    rmax = jnp.max(bv, axis=0, keepdims=True)
    cand = jnp.where(bv == rmax, bi, _S)
    sel = jnp.min(cand)
    sel = jnp.clip(sel, 0, _S - 1)
    gate_r = jax.nn.sigmoid(rmax[:, 0:1])

    cls = pl.ds(sel % 8, 1)
    xs = jnp.broadcast_to(brow_v[0, cls, :].astype(_BF), (16, _D))
    def gate_up(i):
        cols = pl.ds(i * _FC, _FC)
        return (jnp.dot(xs, wg_v[:, cols], preferred_element_type=_F32),
                jnp.dot(xs, wu_v[:, cols], preferred_element_type=_F32))

    y = None
    nxt = gate_up(0)
    for i in range(_F // _FC):
        g, u = nxt
        if i + 1 < _F // _FC:
            nxt = gate_up(i + 1)
        act = (g * jax.nn.sigmoid(g) * u).astype(_BF)
        part = jnp.dot(act, wd_v[pl.ds(i * _FC, _FC), :], preferred_element_type=_F32)
        y = part if y is None else y + part
    y = y[0:1, :]
    row = brow_v[1, cls, :] + modr(5) * (y * gate_r)

    base = pl.multiple_of((sel // 16) * 16, 16)
    rid = base + lax.broadcasted_iota(jnp.int32, (16, _D), 0)
    fix_v[...] = jnp.where(rid == sel, row, out_v[pl.ds(base, 16), :].astype(_F32)).astype(_BF)

    pltpu.make_async_copy(out_v, out_hbm, sems.at[_SEM_OUT]).wait()
    d_fix = cp(fix_v, out_hbm.at[pl.ds(base, 16)], _SEM_FIX)
    d_fix.start()
    d_fix.wait()


@jax.jit
def pallas_adaLN_cond__sliding_block_cached__moe_arch_mod__prompt_kernel(
    A_x: jax.Array,
    A_k_cache: jax.Array,
    A_v_cache: jax.Array,
    A_wq: jax.Array,
    A_wo: jax.Array,
    B_x: jax.Array,
    B_w_r: jax.Array,
    B_w_gate: jax.Array,
    B_w_up: jax.Array,
    B_w_down: jax.Array,
    c: jax.Array,
    w_mod: jax.Array,
):
    del B_x
    x = A_x.reshape(_S, _D)
    k = A_k_cache.reshape(_HKV, _SK, _DH)
    v = A_v_cache.reshape(_HKV, _SK, _DH)

    any_spec = pl.BlockSpec(memory_space=pl.ANY)
    out = pl.pallas_call(
        _kernel,
        out_shape=jax.ShapeDtypeStruct((_S, _D), _BF),
        in_specs=[any_spec] * 11,
        out_specs=any_spec,
        scratch_shapes=[
            pltpu.VMEM((_S, _D), _BF),
            pltpu.VMEM((_M // 2, _D), jnp.uint32),
            pltpu.VMEM((_M // 2, _D), jnp.uint32),
            pltpu.VMEM((_HKV, _W, _DH), _BF),
            pltpu.VMEM((_HKV, _W, _DH), _BF),
            pltpu.VMEM((_NS, _D, _QC), _BF),
            pltpu.VMEM((_NS, _HQ * _DH, _NT), _BF),
            pltpu.VMEM((_NMC, _D, _MC), _BF),
            pltpu.VMEM((_D, _F), _BF),
            pltpu.VMEM((_D, _F), _BF),
            pltpu.VMEM((_F, _D), _BF),
            pltpu.VMEM((1, _D), _BF),
            pltpu.VMEM((_D,), _BF),
            pltpu.VMEM((1, _D), _F32),
            pltpu.VMEM((_NOC, _M // 2, _OW), jnp.uint32),
            pltpu.VMEM((_NOC, _M // 2, _OW), jnp.uint32),
            pltpu.VMEM((_NS, _M, _NT), _F32),
            pltpu.VMEM((_NS, _M, _NT), _F32),
            pltpu.VMEM((_S, _D), _BF),
            pltpu.VMEM((2, 8, _D), _F32),
            pltpu.VMEM((_NMC, 8, _MC), _F32),
            pltpu.VMEM((2, _D), _F32),
            pltpu.VMEM((_D, 128), _F32),
            pltpu.VMEM((8, 128), _F32),
            pltpu.VMEM((8, 128), jnp.int32),
            pltpu.VMEM((16, _D), _BF),
            pltpu.SemaphoreType.DMA((_NSEM,)),
        ],
        compiler_params=pltpu.CompilerParams(vmem_limit_bytes=110 * 1024 * 1024),
    )(x, k, v, A_wq, A_wo, B_w_r, B_w_gate, B_w_up, B_w_down, c, w_mod)
    return out.reshape(1, _S, _D)
```

```python
import functools

import jax
import jax.numpy as jnp
from jax import lax
from jax.experimental import pallas as pl
from jax.experimental.pallas import tpu as pltpu

_S = 2048
_D = 1024
_HQ = 32
_HKV = 4
_DH = 128
_SK = 2048
_W = min(4096, max(256, _SK // 4))
_F = 3584
_EPS = 1e-5

_M = 512
_NB = _S // _M
_HPS = 4
_NS = _HQ // _HPS
_R = _M // _NS
_QC = _HPS * _DH
_NT = _D // _NS
_SPG = _NS // _HKV
_OW = 512
_NOC = _HQ * _DH // _OW
_HPC = _OW // _DH
_TIE_Q = 1
_TIE_D = ((2, 1), (None, 2))
_FC = 256
_MC = 512
_NMC = 6 * _D // _MC
_NMA = 2 * _D // _MC
assert (_NMC - _NMA) % _NS == 0

_LOG2E = 1.4426950408889634
_QSCALE = (_DH ** -0.5) * _LOG2E

_BF = jnp.bfloat16
_F32 = jnp.float32

_SEM_C, _SEM_WR, _SEM_MODB, _SEM_WO, _SEM_WG, _SEM_WU, _SEM_WD = 0, 1, 2, 3, 4, 5, 6
_SEM_OUT, _SEM_FIX = 7, 8
_SEM_WQ = 9
_SEM_X = _SEM_WQ + _NS
_SEM_X1 = _SEM_X + _NB
_SEM_K = _SEM_X1 + _NS
_SEM_V = _SEM_K + _HKV
_SEM_MODA = _SEM_V + _HKV
_NSEM = _SEM_MODA + _NMA


def _kernel(x_hbm, k_hbm, v_hbm, wq_hbm, wo_hbm, wr_hbm, wg_hbm, wu_hbm, wd_hbm, c_hbm, wmod_hbm,
            out_hbm,
            x_v, h_a, h_b, k_v, v_v, wq_v, wo_v, wmod_v, wg_v, wu_v, wd_v, c_v, wr_v, wrf_v,
            o_a, o_b, a_a, a_b, out_v, brow_v, mod_v, modq_v, scol_v, best_v, bidx_v, fix_v, sems):
    h_buf, o_buf, a_buf = (h_a, h_b), (o_a, o_b), (a_a, a_b)

    def cp(src, dst, slot):
        return pltpu.make_async_copy(src, dst, sems.at[slot])

    d_c = cp(c_hbm, c_v, _SEM_C)

    def d_mod(i):
        return cp(wmod_hbm.at[:, pl.ds(i * _MC, _MC)], wmod_v.at[i],
                  _SEM_MODA + i if i < _NMA else _SEM_MODB)

    def d_k(g):
        return cp(k_hbm.at[g, pl.ds(_SK - _W, _W), :], k_v.at[g], _SEM_K + g)

    def d_v(g):
        return cp(v_hbm.at[g, pl.ds(_SK - _W, _W), :], v_v.at[g], _SEM_V + g)

    def d_x1(i):
        rows = pl.ds(pl.multiple_of(_M + i * _R, _R), _R)
        return cp(x_hbm.at[rows], x_v.at[rows], _SEM_X1 + i)

    def d_wq(j):
        return cp(wq_hbm.at[:, pl.ds(pl.multiple_of(j * _QC, _QC), _QC)], wq_v.at[j], _SEM_WQ + j)

    def d_x(b):
        return cp(x_hbm.at[pl.ds(b * _M, _M)], x_v.at[pl.ds(b * _M, _M)], _SEM_X + b)

    d_wr = cp(wr_hbm, wr_v, _SEM_WR)
    d_wg = cp(wg_hbm, wg_v, _SEM_WG)
    d_wu = cp(wu_hbm, wu_v, _SEM_WU)
    d_wd = cp(wd_hbm, wd_v, _SEM_WD)

    d_c.start()
    for i in range(_NMA):
        d_mod(i).start()
    d_x(0).start()
    for j in range(_NS):
        if j % _SPG == 0:
            d_k(j // _SPG).start()
            d_v(j // _SPG).start()
        d_wq(j).start()
        d_x1(j).start()
    for j in range(_NS):
        cp(wo_hbm.at[:, pl.ds(j * _NT, _NT)], wo_v.at[j], _SEM_WO).start()
    for b in range(2, _NB):
        d_x(b).start()
    d_wr.start()
    for i in range(_NMA, _NMC):
        d_mod(i).start()
    d_wg.start()
    d_wu.start()
    d_wd.start()

    def mod_chunk(i):
        cf = c_v[...].astype(_F32)
        sc = jnp.broadcast_to((cf * jax.nn.sigmoid(cf)).astype(_BF), (16, _D))
        m = jnp.dot(sc, wmod_v[i], preferred_element_type=_F32)
        mod_v[i] = m[0:8, :]

    def mod_chunk_vpu(i):
        col = scol_v[...]
        outs = []
        for t in range(_MC // 128):
            w = wmod_v[i, :, pl.ds(t * 128, 128)].astype(_F32)
            outs.append(jnp.sum(w * col, axis=0, keepdims=True))
        mod_v[i, 0:1, :] = jnp.concatenate(outs, axis=1)

    def modr(i):
        n = _D // _MC
        return jnp.concatenate([mod_v[n * i + u, 0:1, :] for u in range(n)], axis=1)

    def pack(xf):
        return pltpu.bitcast(xf.astype(_BF), jnp.uint32)

    def unpack(w):
        return pltpu.bitcast(w, _BF)

    def ln(xf):
        mu = jnp.mean(xf, axis=1, keepdims=True)
        d = xf - mu
        var = jnp.mean(d * d, axis=1, keepdims=True)
        return d * lax.rsqrt(var + _EPS)

    def ln1_slice(b, i):
        rows = pl.ds(pl.multiple_of(b * _M + i * _R, _R), _R)
        y = ln(x_v[rows, :].astype(_F32))
        h = y * modq_v[1:2, :] + modq_v[0:1, :]
        h_buf[b % 2][pl.ds(pl.multiple_of(i * (_R // 2), _R // 2), _R // 2), :] = pack(h)

    def tie(w, token):
        if token is None:
            return w
        return jnp.concatenate([w[0:8, 0:128] | token, w[0:8, 128:]], axis=1) if w.shape[0] == 8 else \
            jnp.concatenate([jnp.concatenate([w[0:8, 0:128] | token, w[0:8, 128:]], axis=1), w[8:]], axis=0)

    def qproj_head(b, j, hh, token=None):
        q = jnp.dot(unpack(tie(h_buf[b % 2][...], token)), wq_v[j, :, pl.ds(hh * _DH, _DH)],
                    preferred_element_type=_F32)
        return q.astype(_BF)

    def scores(j, q):
        return lax.dot_general(q, k_v[j // _SPG], (((1,), (1,)), ((), ())),
                               preferred_element_type=_F32)

    def softmax_pv(b, j, hh, s):
        m = jnp.max(s, axis=1, keepdims=True)
        p = jnp.exp2(s - m)
        l = jnp.sum(p, axis=1, keepdims=True)
        o = jnp.dot(p.astype(_BF), v_v[j // _SPG], preferred_element_type=_F32)
        r = pl.reciprocal(l, approx=True)
        r = r * (2.0 - l * r)
        o_buf[b % 2][j * (_HPS // _HPC) + hh // _HPC, :, pl.ds((hh % _HPC) * _DH, _DH)] = pack(o * r)

    def oproj_part(b, j, part, token=None):
        n = _NOC // _HPS
        lhs = jnp.concatenate([unpack(tie(o_buf[b % 2][part * n + jj], token if jj == 0 else None))
                               for jj in range(n)], axis=1)
        return jnp.dot(lhs, wo_v[j, pl.ds(part * n * _OW, n * _OW), :], preferred_element_type=_F32)

    def epilogue(b, i):
        lrows = pl.ds(pl.multiple_of(i * _R, _R), _R)
        row0 = pl.multiple_of(b * _M + i * _R, _R)
        rows = pl.ds(row0, _R)
        a = jnp.concatenate([a_buf[b % 2][jj, lrows, :] for jj in range(_NS)], axis=1)
        x1 = x_v[rows, :].astype(_F32) + modr(2) * a
        h2 = ln(x1) * (1.0 + modr(4)) + modr(3)
        o = x1 + modr(5) * h2
        out_v[rows, :] = o.astype(_BF)
        r = jnp.sum(h2 * wrf_v[...], axis=1, keepdims=True)
        r = jnp.broadcast_to(r, (_R, 128))
        ridx = row0 + lax.broadcasted_iota(jnp.int32, (_R, 128), 0)
        bv = best_v[...]
        bi = bidx_v[...]
        bh = brow_v[0]
        bo = brow_v[1]
        for s in range(_R // 8):
            grp = slice(s * 8, (s + 1) * 8)
            upd = r[grp] > bv
            bv = jnp.where(upd, r[grp], bv)
            bi = jnp.where(upd, ridx[grp], bi)
            upd_w = jnp.concatenate([upd] * (_D // 128), axis=1)
            bh = jnp.where(upd_w, h2[grp], bh)
            bo = jnp.where(upd_w, o[grp], bo)
        best_v[...] = bv
        bidx_v[...] = bi
        brow_v[0] = bh
        brow_v[1] = bo
        return lax.shift_right_logical(bi, 31).astype(jnp.uint32)

    def block_phase(b):
        do_o = b >= 1
        do_epi = b >= 2
        do_ln = b + 1 < _NB

        def step(j, carry):
            token = None
            if do_epi:
                token = epilogue(b - 2, j)
            if b == 0:
                @pl.when(j % _SPG == 0)
                def _():
                    d_k(j // _SPG).wait()
                    d_v(j // _SPG).wait()
                d_wq(j).wait()
                d_x1(j).wait()
            parts = []
            q = qproj_head(b, j, 0)
            if do_o:
                parts.append(oproj_part(b - 1, j, 0))
            for hh in range(_HPS):
                s = scores(j, q)
                if hh + 1 < _HPS:
                    q = qproj_head(b, j, hh + 1, token if hh + 1 == _TIE_Q else None)
                elif do_o:
                    parts.append(oproj_part(b - 1, j, len(parts)))
                softmax_pv(b, j, hh, s)
            if b == 1:
                for u in range((_NMC - _NMA) // _NS):
                    mod_chunk_vpu(_NMA + j * ((_NMC - _NMA) // _NS) + u)
            if do_ln:
                ln1_slice(b + 1, j)
            if do_o:
                for part in range(len(parts), _HPS):
                    parts.append(oproj_part(b - 1, j, part))
                a_buf[(b - 1) % 2][j] = functools.reduce(lambda u, w: u + w, parts)
            return carry
        lax.fori_loop(0, _NS, step, 0, unroll=1)

    def drain_phase(half):
        b = _NB - 1
        hm = _M // 2

        def step(jp, carry):
            if half == 0:
                tokens = [epilogue(b - 1, 2 * jp + u) for u in range(2)]
            else:
                tokens = [None, epilogue(b, jp)]
            rows_w = pl.ds(half * (hm // 2), hm // 2)
            n = _NOC // _HPS
            for u in range(2):
                j = 2 * jp + u
                parts = []
                for part in range(_HPS):
                    tk = tokens[u] if part == _TIE_D[half][u] else None
                    lhs = jnp.concatenate(
                        [unpack(tie(o_buf[b % 2][part * n + jj, rows_w, :], tk if jj == 0 else None))
                         for jj in range(n)], axis=1)
                    parts.append(jnp.dot(lhs, wo_v[j, pl.ds(part * n * _OW, n * _OW), :],
                                         preferred_element_type=_F32))
                a_buf[b % 2][j, pl.ds(half * hm, hm), :] = functools.reduce(lambda x_, y_: x_ + y_, parts)
            return carry
        lax.fori_loop(0, _NS // 2, step, 0)

    def out_copy(b):
        rows = pl.ds(b * _M, _M)
        return cp(out_v.at[rows], out_hbm.at[rows], _SEM_OUT)

    d_c.wait()
    cf = c_v[...].astype(_F32)
    sc = (cf * jax.nn.sigmoid(cf)).astype(_BF).astype(_F32)
    scol_v[...] = jnp.broadcast_to(sc, (128, _D)).T
    for i in range(_NMA):
        d_mod(i).wait()
        mod_chunk(i)
    modq_v[0:1, :] = modr(0) * _QSCALE
    modq_v[1:2, :] = (1.0 + modr(1)) * _QSCALE
    d_x(0).wait()
    for i in range(_NS):
        ln1_slice(0, i)
    best_v[...] = jnp.full((8, 128), -jnp.inf, _F32)
    bidx_v[...] = jnp.zeros((8, 128), jnp.int32)
    brow_v[...] = jnp.zeros((2, 8, _D), _F32)

    for b in range(_NB):
        if b == 1:
            pltpu.make_async_copy(wo_v, wo_v, sems.at[_SEM_WO]).wait()
            d_wr.wait()
            wrf_v[...] = wr_v[...].astype(_F32).reshape(1, _D)
            pltpu.make_async_copy(wmod_v.at[pl.ds(_NMA, _NMC - _NMA)],
                                  wmod_v.at[pl.ds(_NMA, _NMC - _NMA)], sems.at[_SEM_MODB]).wait()
        if 2 <= b + 1 < _NB:
            d_x(b + 1).wait()
        block_phase(b)
        if b >= 2:
            out_copy(b - 2).start()
    drain_phase(0)
    out_copy(_NB - 2).start()
    d_wg.wait()
    d_wu.wait()
    d_wd.wait()
    drain_phase(1)
    for i in range(_NS // 2, _NS):
        epilogue(_NB - 1, i)
    out_copy(_NB - 1).start()

    bv = best_v[...]
    bi = bidx_v[...]
    rmax = jnp.max(bv, axis=0, keepdims=True)
    cand = jnp.where(bv == rmax, bi, _S)
    sel = jnp.min(cand)
    sel = jnp.clip(sel, 0, _S - 1)
    gate_r = jax.nn.sigmoid(rmax[:, 0:1])

    cls = pl.ds(sel % 8, 1)
    xs = jnp.broadcast_to(brow_v[0, cls, :].astype(_BF), (16, _D))
    def gate_up(i):
        cols = pl.ds(i * _FC, _FC)
        return (jnp.dot(xs, wg_v[:, cols], preferred_element_type=_F32),
                jnp.dot(xs, wu_v[:, cols], preferred_element_type=_F32))

    y = None
    nxt = gate_up(0)
    for i in range(_F // _FC):
        g, u = nxt
        if i + 1 < _F // _FC:
            nxt = gate_up(i + 1)
        act = (g * jax.nn.sigmoid(g) * u).astype(_BF)
        part = jnp.dot(act, wd_v[pl.ds(i * _FC, _FC), :], preferred_element_type=_F32)
        y = part if y is None else y + part
    y = y[0:1, :]
    row = brow_v[1, cls, :] + modr(5) * (y * gate_r)

    base = pl.multiple_of((sel // 16) * 16, 16)
    rid = base + lax.broadcasted_iota(jnp.int32, (16, _D), 0)
    fix_v[...] = jnp.where(rid == sel, row, out_v[pl.ds(base, 16), :].astype(_F32)).astype(_BF)

    pltpu.make_async_copy(out_v, out_hbm, sems.at[_SEM_OUT]).wait()
    d_fix = cp(fix_v, out_hbm.at[pl.ds(base, 16)], _SEM_FIX)
    d_fix.start()
    d_fix.wait()


@jax.jit
def pallas_adaLN_cond__sliding_block_cached__moe_arch_mod__prompt_kernel(
    A_x: jax.Array,
    A_k_cache: jax.Array,
    A_v_cache: jax.Array,
    A_wq: jax.Array,
    A_wo: jax.Array,
    B_x: jax.Array,
    B_w_r: jax.Array,
    B_w_gate: jax.Array,
    B_w_up: jax.Array,
    B_w_down: jax.Array,
    c: jax.Array,
    w_mod: jax.Array,
):
    del B_x
    x = A_x.reshape(_S, _D)
    k = A_k_cache.reshape(_HKV, _SK, _DH)
    v = A_v_cache.reshape(_HKV, _SK, _DH)

    any_spec = pl.BlockSpec(memory_space=pl.ANY)
    out = pl.pallas_call(
        _kernel,
        out_shape=jax.ShapeDtypeStruct((_S, _D), _BF),
        in_specs=[any_spec] * 11,
        out_specs=any_spec,
        scratch_shapes=[
            pltpu.VMEM((_S, _D), _BF),
            pltpu.VMEM((_M // 2, _D), jnp.uint32),
            pltpu.VMEM((_M // 2, _D), jnp.uint32),
            pltpu.VMEM((_HKV, _W, _DH), _BF),
            pltpu.VMEM((_HKV, _W, _DH), _BF),
            pltpu.VMEM((_NS, _D, _QC), _BF),
            pltpu.VMEM((_NS, _HQ * _DH, _NT), _BF),
            pltpu.VMEM((_NMC, _D, _MC), _BF),
            pltpu.VMEM((_D, _F), _BF),
            pltpu.VMEM((_D, _F), _BF),
            pltpu.VMEM((_F, _D), _BF),
            pltpu.VMEM((1, _D), _BF),
            pltpu.VMEM((_D,), _BF),
            pltpu.VMEM((1, _D), _F32),
            pltpu.VMEM((_NOC, _M // 2, _OW), jnp.uint32),
            pltpu.VMEM((_NOC, _M // 2, _OW), jnp.uint32),
            pltpu.VMEM((_NS, _M, _NT), _F32),
            pltpu.VMEM((_NS, _M, _NT), _F32),
            pltpu.VMEM((_S, _D), _BF),
            pltpu.VMEM((2, 8, _D), _F32),
            pltpu.VMEM((_NMC, 8, _MC), _F32),
            pltpu.VMEM((2, _D), _F32),
            pltpu.VMEM((_D, 128), _F32),
            pltpu.VMEM((8, 128), _F32),
            pltpu.VMEM((8, 128), jnp.int32),
            pltpu.VMEM((16, _D), _BF),
            pltpu.SemaphoreType.DMA((_NSEM,)),
        ],
        compiler_params=pltpu.CompilerParams(vmem_limit_bytes=110 * 1024 * 1024),
    )(x, k, v, A_wq, A_wo, B_w_r, B_w_gate, B_w_up, B_w_down, c, w_mod)
    return out.reshape(1, _S, _D)
```

```python
import functools

import jax
import jax.numpy as jnp
from jax import lax
from jax.experimental import pallas as pl
from jax.experimental.pallas import tpu as pltpu

_S = 2048
_D = 1024
_HQ = 32
_HKV = 4
_DH = 128
_SK = 2048
_W = min(4096, max(256, _SK // 4))
_F = 3584
_EPS = 1e-5

_M = 512
_NB = _S // _M
_HPS = 4
_NS = _HQ // _HPS
_R = _M // _NS
_QC = _HPS * _DH
_NT = _D // _NS
_SPG = _NS // _HKV
_OW = 512
_NOC = _HQ * _DH // _OW
_HPC = _OW // _DH
_TIE_Q = 1
_TIE_D = ((2, 1), (None, 2))
_FC = 256
_MC = 512
_NMC = 6 * _D // _MC
_NMA = 2 * _D // _MC
assert (_NMC - _NMA) % _NS == 0

_LOG2E = 1.4426950408889634
_QSCALE = (_DH ** -0.5) * _LOG2E

_BF = jnp.bfloat16
_F32 = jnp.float32

_SEM_C, _SEM_WR, _SEM_MODB, _SEM_WO, _SEM_WG, _SEM_WU, _SEM_WD = 0, 1, 2, 3, 4, 5, 6
_SEM_OUT, _SEM_FIX = 7, 8
_SEM_WQ = 9
_SEM_X = _SEM_WQ + _NS
_SEM_X1 = _SEM_X + _NB
_SEM_K = _SEM_X1 + _NS
_SEM_V = _SEM_K + _HKV
_SEM_MODA = _SEM_V + _HKV
_NSEM = _SEM_MODA + _NMA


def _kernel(x_hbm, k_hbm, v_hbm, wq_hbm, wo_hbm, wr_hbm, wg_hbm, wu_hbm, wd_hbm, c_hbm, wmod_hbm,
            out_hbm,
            x_v, h_a, h_b, k_v, v_v, wq_v, wo_v, wmod_v, wg_v, wu_v, wd_v, c_v, wr_v, wrf_v,
            o_a, o_b, a_a, a_b, out_v, brow_v, mod_v, modq_v, scol_v, best_v, bidx_v, fix_v, sems):
    h_buf, o_buf, a_buf = (h_a, h_b), (o_a, o_b), (a_a, a_b)

    def cp(src, dst, slot):
        return pltpu.make_async_copy(src, dst, sems.at[slot])

    d_c = cp(c_hbm, c_v, _SEM_C)

    def d_mod(i):
        return cp(wmod_hbm.at[:, pl.ds(i * _MC, _MC)], wmod_v.at[i],
                  _SEM_MODA + i if i < _NMA else _SEM_MODB)

    def d_k(g):
        return cp(k_hbm.at[g, pl.ds(_SK - _W, _W), :], k_v.at[g], _SEM_K + g)

    def d_v(g):
        return cp(v_hbm.at[g, pl.ds(_SK - _W, _W), :], v_v.at[g], _SEM_V + g)

    def d_x1(i):
        rows = pl.ds(pl.multiple_of(_M + i * _R, _R), _R)
        return cp(x_hbm.at[rows], x_v.at[rows], _SEM_X1 + i)

    def d_wq(j):
        return cp(wq_hbm.at[:, pl.ds(pl.multiple_of(j * _QC, _QC), _QC)], wq_v.at[j], _SEM_WQ + j)

    def d_x(b):
        return cp(x_hbm.at[pl.ds(b * _M, _M)], x_v.at[pl.ds(b * _M, _M)], _SEM_X + b)

    d_wr = cp(wr_hbm, wr_v, _SEM_WR)
    d_wg = cp(wg_hbm, wg_v, _SEM_WG)
    d_wu = cp(wu_hbm, wu_v, _SEM_WU)
    d_wd = cp(wd_hbm, wd_v, _SEM_WD)

    d_c.start()
    for i in range(_NMA):
        d_mod(i).start()
    d_x(0).start()
    for j in range(_NS):
        if j % _SPG == 0:
            d_k(j // _SPG).start()
            d_v(j // _SPG).start()
        d_wq(j).start()
        d_x1(j).start()
    for j in range(_NS):
        cp(wo_hbm.at[:, pl.ds(j * _NT, _NT)], wo_v.at[j], _SEM_WO).start()
    for b in range(2, _NB):
        d_x(b).start()
    d_wr.start()
    for i in range(_NMA, _NMC):
        d_mod(i).start()
    d_wg.start()
    d_wu.start()
    d_wd.start()

    def mod_chunk(i):
        cf = c_v[...].astype(_F32)
        sc = jnp.broadcast_to((cf * jax.nn.sigmoid(cf)).astype(_BF), (16, _D))
        m = jnp.dot(sc, wmod_v[i], preferred_element_type=_F32)
        mod_v[i] = m[0:8, :]

    def mod_chunk_vpu(i):
        col = scol_v[...]
        outs = []
        for t in range(_MC // 128):
            w = wmod_v[i, :, pl.ds(t * 128, 128)].astype(_F32)
            outs.append(jnp.sum(w * col, axis=0, keepdims=True))
        mod_v[i, 0:1, :] = jnp.concatenate(outs, axis=1)

    def modr(i):
        n = _D // _MC
        return jnp.concatenate([mod_v[n * i + u, 0:1, :] for u in range(n)], axis=1)

    def pack(xf):
        return pltpu.bitcast(xf.astype(_BF), jnp.uint32)

    def unpack(w):
        return pltpu.bitcast(w, _BF)

    def ln(xf):
        mu = jnp.mean(xf, axis=1, keepdims=True)
        d = xf - mu
        var = jnp.mean(d * d, axis=1, keepdims=True)
        return d * lax.rsqrt(var + _EPS)

    def ln1_slice(b, i):
        rows = pl.ds(pl.multiple_of(b * _M + i * _R, _R), _R)
        y = ln(x_v[rows, :].astype(_F32))
        h = y * modq_v[1:2, :] + modq_v[0:1, :]
        h_buf[b % 2][pl.ds(pl.multiple_of(i * (_R // 2), _R // 2), _R // 2), :] = pack(h)

    def tie(w, token):
        if token is None:
            return w
        return jnp.concatenate([w[0:8, 0:128] | token, w[0:8, 128:]], axis=1) if w.shape[0] == 8 else \
            jnp.concatenate([jnp.concatenate([w[0:8, 0:128] | token, w[0:8, 128:]], axis=1), w[8:]], axis=0)

    def qproj_head(b, j, hh, token=None):
        q = jnp.dot(unpack(tie(h_buf[b % 2][...], token)), wq_v[j, :, pl.ds(hh * _DH, _DH)],
                    preferred_element_type=_F32)
        return q.astype(_BF)

    def scores(j, q):
        return lax.dot_general(q, k_v[j // _SPG], (((1,), (1,)), ((), ())),
                               preferred_element_type=_F32)

    def softmax_pv(b, j, hh, s):
        m = jnp.max(s, axis=1, keepdims=True)
        p = jnp.exp2(s - m)
        l = jnp.sum(p, axis=1, keepdims=True)
        o = jnp.dot(p.astype(_BF), v_v[j // _SPG], preferred_element_type=_F32)
        r = pl.reciprocal(l, approx=True)
        r = r * (2.0 - l * r)
        o_buf[b % 2][j * (_HPS // _HPC) + hh // _HPC, :, pl.ds((hh % _HPC) * _DH, _DH)] = pack(o * r)

    def oproj_part(b, j, part, token=None):
        n = _NOC // _HPS
        lhs = jnp.concatenate([unpack(tie(o_buf[b % 2][part * n + jj], token if jj == 0 else None))
                               for jj in range(n)], axis=1)
        return jnp.dot(lhs, wo_v[j, pl.ds(part * n * _OW, n * _OW), :], preferred_element_type=_F32)

    def epilogue(b, i):
        lrows = pl.ds(pl.multiple_of(i * _R, _R), _R)
        row0 = pl.multiple_of(b * _M + i * _R, _R)
        rows = pl.ds(row0, _R)
        a = jnp.concatenate([a_buf[b % 2][jj, lrows, :] for jj in range(_NS)], axis=1)
        x1 = x_v[rows, :].astype(_F32) + modr(2) * a
        h2 = ln(x1) * (1.0 + modr(4)) + modr(3)
        o = x1 + modr(5) * h2
        out_v[rows, :] = o.astype(_BF)
        r = jnp.sum(h2 * wrf_v[...], axis=1, keepdims=True)
        r = jnp.broadcast_to(r, (_R, 128))
        ridx = row0 + lax.broadcasted_iota(jnp.int32, (_R, 128), 0)
        bv = best_v[...]
        bi = bidx_v[...]
        bh = brow_v[0]
        bo = brow_v[1]
        for s in range(_R // 8):
            grp = slice(s * 8, (s + 1) * 8)
            upd = r[grp] > bv
            bv = jnp.where(upd, r[grp], bv)
            bi = jnp.where(upd, ridx[grp], bi)
            upd_w = jnp.concatenate([upd] * (_D // 128), axis=1)
            bh = jnp.where(upd_w, h2[grp], bh)
            bo = jnp.where(upd_w, o[grp], bo)
        best_v[...] = bv
        bidx_v[...] = bi
        brow_v[0] = bh
        brow_v[1] = bo
        return lax.shift_right_logical(bi, 31).astype(jnp.uint32)

    def block_phase(b):
        do_o = b >= 1
        do_epi = b >= 2
        do_ln = b + 1 < _NB

        def step(j, carry):
            token = None
            if do_epi:
                token = epilogue(b - 2, j)
            if b == 0:
                @pl.when(j % _SPG == 0)
                def _():
                    d_k(j // _SPG).wait()
                    d_v(j // _SPG).wait()
                d_wq(j).wait()
                d_x1(j).wait()
            parts = []
            q = qproj_head(b, j, 0)
            if do_o:
                parts.append(oproj_part(b - 1, j, 0))
            for hh in range(_HPS):
                s = scores(j, q)
                if hh + 1 < _HPS:
                    q = qproj_head(b, j, hh + 1, token if hh + 1 == _TIE_Q else None)
                elif do_o:
                    parts.append(oproj_part(b - 1, j, len(parts)))
                softmax_pv(b, j, hh, s)
            if b == 1:
                for u in range((_NMC - _NMA) // _NS):
                    mod_chunk_vpu(_NMA + j * ((_NMC - _NMA) // _NS) + u)
            if do_ln:
                ln1_slice(b + 1, j)
            if do_o:
                for part in range(len(parts), _HPS):
                    parts.append(oproj_part(b - 1, j, part))
                a_buf[(b - 1) % 2][j] = functools.reduce(lambda u, w: u + w, parts)
            return carry
        lax.fori_loop(0, _NS, step, 0, unroll=1)

    def drain_phase(half):
        b = _NB - 1
        hm = _M // 2

        def step(jp, carry):
            if half == 0:
                tokens = [epilogue(b - 1, 2 * jp + u) for u in range(2)]
            else:
                tokens = [None, epilogue(b, jp)]
            rows_w = pl.ds(half * (hm // 2), hm // 2)
            n = _NOC // _HPS
            for u in range(2):
                j = 2 * jp + u
                parts = []
                for part in range(_HPS):
                    tk = tokens[u] if part == _TIE_D[half][u] else None
                    lhs = jnp.concatenate(
                        [unpack(tie(o_buf[b % 2][part * n + jj, rows_w, :], tk if jj == 0 else None))
                         for jj in range(n)], axis=1)
                    parts.append(jnp.dot(lhs, wo_v[j, pl.ds(part * n * _OW, n * _OW), :],
                                         preferred_element_type=_F32))
                a_buf[b % 2][j, pl.ds(half * hm, hm), :] = functools.reduce(lambda x_, y_: x_ + y_, parts)
            return carry
        lax.fori_loop(0, _NS // 2, step, 0)

    def out_copy(b):
        rows = pl.ds(b * _M, _M)
        return cp(out_v.at[rows], out_hbm.at[rows], _SEM_OUT)

    d_c.wait()
    cf = c_v[...].astype(_F32)
    sc = (cf * jax.nn.sigmoid(cf)).astype(_BF).astype(_F32)
    scol_v[...] = jnp.broadcast_to(sc, (128, _D)).T
    for i in range(_NMA):
        d_mod(i).wait()
        mod_chunk(i)
    modq_v[0:1, :] = modr(0) * _QSCALE
    modq_v[1:2, :] = (1.0 + modr(1)) * _QSCALE
    d_x(0).wait()
    for i in range(_NS):
        ln1_slice(0, i)
    best_v[...] = jnp.full((8, 128), -jnp.inf, _F32)
    bidx_v[...] = jnp.zeros((8, 128), jnp.int32)
    brow_v[...] = jnp.zeros((2, 8, _D), _F32)

    for b in range(_NB):
        if b == 1:
            pltpu.make_async_copy(wo_v, wo_v, sems.at[_SEM_WO]).wait()
            d_wr.wait()
            wrf_v[...] = wr_v[...].astype(_F32).reshape(1, _D)
            pltpu.make_async_copy(wmod_v.at[pl.ds(_NMA, _NMC - _NMA)],
                                  wmod_v.at[pl.ds(_NMA, _NMC - _NMA)], sems.at[_SEM_MODB]).wait()
        if 2 <= b + 1 < _NB:
            d_x(b + 1).wait()
        block_phase(b)
        if b >= 2:
            out_copy(b - 2).start()
    drain_phase(0)
    out_copy(_NB - 2).start()
    d_wg.wait()
    d_wu.wait()
    d_wd.wait()
    drain_phase(1)
    for i in range(_NS // 2, _NS):
        epilogue(_NB - 1, i)
    out_copy(_NB - 1).start()

    bv = best_v[...]
    bi = bidx_v[...]
    rmax = jnp.max(bv, axis=0, keepdims=True)
    cand = jnp.where(bv == rmax, bi, _S)
    selv = jnp.min(cand, axis=0, keepdims=True)
    won = jnp.concatenate([cand == selv] * (_D // 128), axis=1)
    gate_r = jax.nn.sigmoid(rmax[:, 0:1])

    def winner_row(k):
        return jnp.sum(jnp.where(won, brow_v[k], 0.0), axis=0, keepdims=True)

    xs = jnp.broadcast_to(winner_row(0).astype(_BF), (16, _D))
    def gate_up(i):
        cols = pl.ds(i * _FC, _FC)
        return (jnp.dot(xs, wg_v[:, cols], preferred_element_type=_F32),
                jnp.dot(xs, wu_v[:, cols], preferred_element_type=_F32))

    y = None
    nxt = gate_up(0)
    for i in range(_F // _FC):
        g, u = nxt
        if i + 1 < _F // _FC:
            nxt = gate_up(i + 1)
        act = (g * jax.nn.sigmoid(g) * u).astype(_BF)
        part = jnp.dot(act, wd_v[pl.ds(i * _FC, _FC), :], preferred_element_type=_F32)
        y = part if y is None else y + part
    y = y[0:1, :]
    row = winner_row(1) + modr(5) * (y * gate_r)

    sel = jnp.clip(jnp.min(cand), 0, _S - 1)

    base = pl.multiple_of((sel // 16) * 16, 16)
    rid = base + lax.broadcasted_iota(jnp.int32, (16, _D), 0)
    fix_v[...] = jnp.where(rid == sel, row, out_v[pl.ds(base, 16), :].astype(_F32)).astype(_BF)

    pltpu.make_async_copy(out_v, out_hbm, sems.at[_SEM_OUT]).wait()
    d_fix = cp(fix_v, out_hbm.at[pl.ds(base, 16)], _SEM_FIX)
    d_fix.start()
    d_fix.wait()


@jax.jit
def pallas_adaLN_cond__sliding_block_cached__moe_arch_mod__prompt_kernel(
    A_x: jax.Array,
    A_k_cache: jax.Array,
    A_v_cache: jax.Array,
    A_wq: jax.Array,
    A_wo: jax.Array,
    B_x: jax.Array,
    B_w_r: jax.Array,
    B_w_gate: jax.Array,
    B_w_up: jax.Array,
    B_w_down: jax.Array,
    c: jax.Array,
    w_mod: jax.Array,
):
    del B_x
    x = A_x.reshape(_S, _D)
    k = A_k_cache.reshape(_HKV, _SK, _DH)
    v = A_v_cache.reshape(_HKV, _SK, _DH)

    any_spec = pl.BlockSpec(memory_space=pl.ANY)
    out = pl.pallas_call(
        _kernel,
        out_shape=jax.ShapeDtypeStruct((_S, _D), _BF),
        in_specs=[any_spec] * 11,
        out_specs=any_spec,
        scratch_shapes=[
            pltpu.VMEM((_S, _D), _BF),
            pltpu.VMEM((_M // 2, _D), jnp.uint32),
            pltpu.VMEM((_M // 2, _D), jnp.uint32),
            pltpu.VMEM((_HKV, _W, _DH), _BF),
            pltpu.VMEM((_HKV, _W, _DH), _BF),
            pltpu.VMEM((_NS, _D, _QC), _BF),
            pltpu.VMEM((_NS, _HQ * _DH, _NT), _BF),
            pltpu.VMEM((_NMC, _D, _MC), _BF),
            pltpu.VMEM((_D, _F), _BF),
            pltpu.VMEM((_D, _F), _BF),
            pltpu.VMEM((_F, _D), _BF),
            pltpu.VMEM((1, _D), _BF),
            pltpu.VMEM((_D,), _BF),
            pltpu.VMEM((1, _D), _F32),
            pltpu.VMEM((_NOC, _M // 2, _OW), jnp.uint32),
            pltpu.VMEM((_NOC, _M // 2, _OW), jnp.uint32),
            pltpu.VMEM((_NS, _M, _NT), _F32),
            pltpu.VMEM((_NS, _M, _NT), _F32),
            pltpu.VMEM((_S, _D), _BF),
            pltpu.VMEM((2, 8, _D), _F32),
            pltpu.VMEM((_NMC, 8, _MC), _F32),
            pltpu.VMEM((2, _D), _F32),
            pltpu.VMEM((_D, 128), _F32),
            pltpu.VMEM((8, 128), _F32),
            pltpu.VMEM((8, 128), jnp.int32),
            pltpu.VMEM((16, _D), _BF),
            pltpu.SemaphoreType.DMA((_NSEM,)),
        ],
        compiler_params=pltpu.CompilerParams(vmem_limit_bytes=110 * 1024 * 1024),
    )(x, k, v, A_wq, A_wo, B_w_r, B_w_gate, B_w_up, B_w_down, c, w_mod)
    return out.reshape(1, _S, _D)
```
